```python
import jax
import jax.numpy as jnp

def _softmax(x, axis=-1):
    return jax.nn.softmax(x, axis=axis)

def _gelu(x):
    return jax.nn.gelu(x, approximate=True)

def _silu(x):
    return jax.nn.silu(x)

def _sigmoid(x):
    return jax.nn.sigmoid(x)

def _layernorm(x, axis=-1, eps=1e-05):
    m = jnp.mean(x, axis=axis, keepdims=True)
    v = jnp.var(x, axis=axis, keepdims=True)
    return (x - m) / jnp.sqrt(v + eps)

def _scatter_add(tgt, idx, src, axis=0):
    return tgt.at[idx].add(src)

def _segment_sum(src, seg, n):
    return jax.ops.segment_sum(src, seg, n)

class _Rng:

    def __init__(self, key):
        self._k = key

    def _next(self):
        self._k, sub = jax.random.split(self._k)
        return sub

    def normal(self, shape):
        return jax.random.normal(self._next(), shape, dtype=jnp.bfloat16)

    def randint(self, lo, hi, shape):
        return jax.random.randint(self._next(), shape, lo, hi, dtype=jnp.int32)

    def uniform(self, shape, lo=0.0, hi=1.0):
        return jax.random.uniform(self._next(), shape, jnp.bfloat16, lo, hi)

    def permutation(self, n):
        return jax.random.permutation(self._next(), n)
kernel_name = 'adaLN_cond__compressed_kv_cla__glu_gated_geglu__decode'

def setup_inputs():
    _rng = _Rng(jax.random.key(int.from_bytes(__import__("os").urandom(4), "little")))
    _w = lambda a: (lambda t: t.astype(jnp.bfloat16) if jnp.issubdtype(t.dtype, jnp.floating) else t)(jnp.asarray(a))

    def _A_setup():
        B, H, Sq, Sk, D, M = (1, 32, 1, 32768, 128, 512)
        Dc = 4 * D
        return {'x': _w((lambda *s: _rng.normal(s) * 0.05)(B, Sq, M)), 'c_kv': _w((lambda *s: _rng.normal(s) * 0.05)(B, Sk, Dc)), 'w_q': _w((lambda *s: _rng.normal(s) * 0.05)(M, H, D) * M ** (-0.5)), 'w_uk': _w((lambda *s: _rng.normal(s) * 0.05)(Dc, H, D) * Dc ** (-0.5)), 'w_uv': _w((lambda *s: _rng.normal(s) * 0.05)(Dc, H, D) * Dc ** (-0.5)), 'w_o': _w((lambda *s: _rng.normal(s) * 0.05)(H, D, M) * (H * D) ** (-0.5))}
    _A_in = _A_setup()

    def _B_setup():
        B, S, Dm, Df = (1, 1, 512, 1792)
        return {'x': _w((lambda *s: _rng.normal(s) * 0.05)(B, S, Dm)), 'w_gate': _w((lambda *s: _rng.normal(s) * 0.05)(Dm, Df) * Dm ** (-0.5)), 'w_up': _w((lambda *s: _rng.normal(s) * 0.05)(Dm, Df) * Dm ** (-0.5)), 'w_down': _w((lambda *s: _rng.normal(s) * 0.05)(Df, Dm) * Df ** (-0.5))}
    _B_in = _B_setup()
    return {'A_x': _A_in['x'], 'A_c_kv': _A_in['c_kv'], 'A_w_q': _A_in['w_q'], 'A_w_uk': _A_in['w_uk'], 'A_w_uv': _A_in['w_uv'], 'A_w_o': _A_in['w_o'], 'B_x': _B_in['x'], 'B_w_gate': _B_in['w_gate'], 'B_w_up': _B_in['w_up'], 'B_w_down': _B_in['w_down'], 'c': _w((lambda *s: _rng.normal(s) * 0.05)(1, 512)), 'w_mod': _w((lambda *s: _rng.normal(s) * 0.05)(512, 6 * 512) * 512 ** (-0.5))}

def reference(A_x, A_c_kv, A_w_q, A_w_uk, A_w_uv, A_w_o, B_x, B_w_gate, B_w_up, B_w_down, c, w_mod):

    def _A_ref(x, c_kv, w_q, w_uk, w_uv, w_o):
        B, Sq, M = (x.shape[0], x.shape[1], x.shape[2])
        Sk = c_kv.shape[1]
        H, D = (w_q.shape[1], w_q.shape[2])
        q = jnp.einsum('bqm,mhd->bhqd', x, w_q)
        k = jnp.einsum('bkc,chd->bhkd', c_kv, w_uk)
        v = jnp.einsum('bkc,chd->bhkd', c_kv, w_uv)
        scores = jnp.einsum('bhqd,bhkd->bhqk', q, k) * D ** (-0.5)
        off = Sk - Sq
        qi = jnp.arange(Sq)[:, None]
        kj = jnp.arange(Sk)[None, :]
        cmask = kj <= qi + off
        scores = jnp.where(cmask[None, None], scores, -1000000000.0)
        p = _softmax(scores, axis=-1)
        ctx = jnp.einsum('bhqk,bhkd->bhqd', p, v)
        return jnp.einsum('bhqd,hdm->bqm', ctx, w_o)

    def _B_ref(x, w_gate, w_up, w_down):
        g = jnp.einsum('bsd,df->bsf', x, w_gate)
        u = jnp.einsum('bsd,df->bsf', x, w_up)
        h = _gelu(g) * u
        return jnp.einsum('bsf,fd->bsd', h, w_down)
    x = A_x
    mod = (_silu(c) @ w_mod).reshape(c.shape[0], 6, 1, -1)
    sa, ca, ga, sb, cb, gb = (mod[:, 0].copy(), mod[:, 1].copy(), mod[:, 2].copy(), mod[:, 3].copy(), mod[:, 4].copy(), mod[:, 5].copy())
    h = _layernorm(x, axis=-1) * (1 + ca) + sa
    x = x + ga * _A_ref(h, A_c_kv, A_w_q, A_w_uk, A_w_uv, A_w_o)
    h = _layernorm(x, axis=-1) * (1 + cb) + sb
    x = x + gb * _B_ref(h, B_w_gate, B_w_up, B_w_down)
    return x
```

```python
import functools

import jax
import jax.numpy as jnp
from jax import lax
import jax.experimental.pallas as pl
import jax.experimental.pallas.tpu as pltpu

_F32 = jnp.float32
_BF16 = jnp.bfloat16
_NT = (((1,), (1,)), ((), ()))
_LANES = 128


def _layernorm(x, eps=1e-05):
    m = jnp.mean(x, axis=-1, keepdims=True)
    xc = x - m
    v = jnp.mean(xc * xc, axis=-1, keepdims=True)
    return xc / jnp.sqrt(v + eps)


def _kernel(
    x_hbm, c_hbm, wmod_hbm, wq_hbm, wuk_hbm, ckv_hbm, wuv_hbm, wo_hbm,
    wg_hbm, wu_hbm, wd_hbm,
    o_ref,
    x_v, c_v, wmod_v, wq_v, wuk_v, ckv_v, wuv_v, wo_v, wg_v, wu_v, wd_v,
    e_v, s_v, sems,
    *, H, D, M, DC, SK, DF, kv_chunks, tk, wd_split,
):
    copies = {}
    order = []

    def add(name, src, dst):
        cp = pltpu.make_async_copy(src, dst, sems.at[len(order)])
        copies[name] = cp
        order.append(name)

    add("x", x_hbm, x_v)
    add("c", c_hbm, c_v)
    add("wmod", wmod_hbm, wmod_v)
    add("wq", wq_hbm, wq_v)
    add("wuk", wuk_hbm, wuk_v)
    kv_starts = []
    r0 = 0
    for i, rows in enumerate(kv_chunks):
        add(f"kv{i}", ckv_hbm.at[pl.ds(r0, rows)], ckv_v.at[pl.ds(r0, rows)])
        kv_starts.append(r0)
        r0 += rows
    add("wuv", wuv_hbm, wuv_v)
    add("wo", wo_hbm, wo_v)
    add("wg", wg_hbm, wg_v)
    add("wu", wu_hbm, wu_v)
    wd_starts = []
    r0 = 0
    for i, rows in enumerate(wd_split):
        add(f"wd{i}", wd_hbm.at[pl.ds(r0, rows)], wd_v.at[pl.ds(r0, rows)])
        wd_starts.append(r0)
        r0 += rows
    for name in order:
        copies[name].start()

    nblk = DC // _LANES
    ew = _LANES * H
    cb = 512
    for j in range(ew // cb):
        row = lax.broadcasted_iota(jnp.int32, (_LANES, cb), 0)
        col = lax.broadcasted_iota(jnp.int32, (_LANES, cb), 1) + j * cb
        e_v[:, j * cb:(j + 1) * cb] = jnp.where(
            col // H == row, 1.0, 0.0).astype(_BF16)

    def head_mask(rows):
        row = lax.broadcasted_iota(jnp.int32, (rows, cb), 0)
        col = lax.broadcasted_iota(jnp.int32, (rows, cb), 1)
        return (col % H) == (row % H)

    def expand(a):
        a4 = jnp.concatenate(
            [jnp.broadcast_to(a[:, u * _LANES:(u + 1) * _LANES], (H, _LANES))
             for u in range(nblk)], axis=0).astype(_BF16)
        mask = head_mask(nblk * H)
        for j in range(ew // cb):
            xj = jnp.dot(a4, e_v[:, j * cb:(j + 1) * cb],
                         preferred_element_type=_F32)
            xj = jnp.where(mask, xj, 0.0).astype(_BF16)
            for u in range(nblk):
                s_v[:, u * ew + j * cb:u * ew + (j + 1) * cb] = (
                    xj[u * H:(u + 1) * H, :])

    def per_head_matvec(w_v):
        parts = [
            jnp.dot(s_v[:, u * ew:(u + 1) * ew], w_v[u * ew:(u + 1) * ew, :],
                    preferred_element_type=_F32)
            for u in range(nblk)
        ]
        return functools.reduce(lambda a, b: a + b, parts)

    copies["x"].wait()
    copies["c"].wait()
    copies["wmod"].wait()
    cc = c_v[...].astype(_F32)
    sc = jnp.broadcast_to(cc * jax.nn.sigmoid(cc), (8, M)).astype(_BF16)
    mod = jnp.dot(sc, wmod_v[...], preferred_element_type=_F32)[0:1, :]
    sa, ca, ga, sb, cb_, gb = (mod[:, i * M:(i + 1) * M] for i in range(6))
    x0 = x_v[...].astype(_F32)
    h1 = _layernorm(x0) * (1.0 + ca) + sa

    expand(h1)
    copies["wq"].wait()
    q = per_head_matvec(wq_v).astype(_BF16)

    copies["wuk"].wait()
    scale = float(D) ** -0.5
    mask = head_mask(H)
    for j in range(DC * H // cb):
        rj = lax.dot_general(q, wuk_v[j * cb:(j + 1) * cb, :], _NT,
                             preferred_element_type=_F32)
        s_v[:, j * cb:(j + 1) * cb] = jnp.where(
            mask, rj * scale, 0.0).astype(_BF16)
    r4 = jnp.concatenate(
        [s_v[:, u * ew:(u + 1) * ew] for u in range(nblk)], axis=0)
    qa4 = lax.dot_general(r4, e_v[...], _NT,
                          preferred_element_type=_F32)
    qa = jnp.concatenate(
        [qa4[u * H:(u + 1) * H, :] for u in range(nblk)], axis=1
    ).astype(_BF16)

    def attn_step(start, carry):
        m, l, acc = carry
        kv = ckv_v[pl.ds(start, tk), :]
        s = lax.dot_general(qa, kv, _NT, preferred_element_type=_F32)
        m_new = jnp.maximum(m, jnp.max(s, axis=1, keepdims=True))
        alpha = jnp.exp(m - m_new)
        p = jnp.exp(s - m_new)
        l = l * alpha + jnp.sum(p, axis=1, keepdims=True)
        acc = acc * alpha + jnp.dot(p.astype(_BF16), kv,
                                    preferred_element_type=_F32)
        return m_new, l, acc

    carry = (jnp.full((H, 1), -jnp.inf, _F32), jnp.zeros((H, 1), _F32),
             jnp.zeros((H, DC), _F32))
    for i, rows in enumerate(kv_chunks):
        copies[f"kv{i}"].wait()
        base = kv_starts[i]
        carry = lax.fori_loop(
            0, rows // tk,
            lambda t, cr, base=base: attn_step(
                pl.multiple_of(base + t * tk, tk), cr),
            carry)
    _, l, acc = carry
    ctx_c = acc / l

    expand(ctx_c)
    copies["wuv"].wait()
    ctx = per_head_matvec(wuv_v)

    row = lax.broadcasted_iota(jnp.int32, (H, D), 0)
    lhs = jnp.concatenate(
        [jnp.where(row == h, ctx, 0.0).astype(_BF16) for h in range(H)],
        axis=1)
    copies["wo"].wait()
    attn = jnp.sum(jnp.dot(lhs, wo_v[...], preferred_element_type=_F32),
                   axis=0, keepdims=True)
    x1 = x0 + ga * attn

    h2 = _layernorm(x1) * (1.0 + cb_) + sb
    h2 = jnp.broadcast_to(h2, (8, M)).astype(_BF16)
    copies["wg"].wait()
    g = jnp.dot(h2, wg_v[...], preferred_element_type=_F32)
    g = jax.nn.gelu(g, approximate=True)
    copies["wu"].wait()
    u = jnp.dot(h2, wu_v[...], preferred_element_type=_F32)
    hf = (g * u).astype(_BF16)
    y = None
    for i, rows in enumerate(wd_split):
        copies[f"wd{i}"].wait()
        r0 = wd_starts[i]
        part = jnp.dot(hf[:, r0:r0 + rows], wd_v[r0:r0 + rows, :],
                       preferred_element_type=_F32)
        y = part if y is None else y + part
    o_ref[...] = (x1 + gb * y[0:1, :]).astype(o_ref.dtype)


@jax.jit
def pallas_adaLN_cond__compressed_kv_cla__glu_gated_geglu__decode_kernel(
    A_x: jax.Array,
    A_c_kv: jax.Array,
    A_w_q: jax.Array,
    A_w_uk: jax.Array,
    A_w_uv: jax.Array,
    A_w_o: jax.Array,
    B_x: jax.Array,
    B_w_gate: jax.Array,
    B_w_up: jax.Array,
    B_w_down: jax.Array,
    c: jax.Array,
    w_mod: jax.Array,
):
    del B_x
    B, SQ, M = A_x.shape
    _, SK, DC = A_c_kv.shape
    _, H, D = A_w_q.shape
    DF = B_w_gate.shape[1]
    assert B == 1 and SQ == 1 and M == DC

    kv_chunks = (SK // 4,) * 4
    tk = 2048
    wd_split = (DF - 256, 256)
    n_dma = 9 + len(kv_chunks) + len(wd_split)

    kernel = functools.partial(
        _kernel, H=H, D=D, M=M, DC=DC, SK=SK, DF=DF,
        kv_chunks=kv_chunks, tk=tk, wd_split=wd_split)

    dt = A_x.dtype
    out = pl.pallas_call(
        kernel,
        out_shape=jax.ShapeDtypeStruct((1, M), dt),
        in_specs=[pl.BlockSpec(memory_space=pl.ANY)] * 11,
        out_specs=pl.BlockSpec(memory_space=pltpu.VMEM),
        scratch_shapes=[
            pltpu.VMEM((1, M), dt),
            pltpu.VMEM((1, M), dt),
            pltpu.VMEM((M, 6 * M), dt),
            pltpu.VMEM((M * H, D), dt),
            pltpu.VMEM((DC * H, D), dt),
            pltpu.VMEM((SK, DC), dt),
            pltpu.VMEM((DC * H, D), dt),
            pltpu.VMEM((H * D, M), dt),
            pltpu.VMEM((M, DF), dt),
            pltpu.VMEM((M, DF), dt),
            pltpu.VMEM((DF, M), dt),
            pltpu.VMEM((_LANES, _LANES * H), _BF16),
            pltpu.VMEM((H, DC * H), _BF16),
            pltpu.SemaphoreType.DMA((n_dma,)),
        ],
        compiler_params=pltpu.CompilerParams(
            vmem_limit_bytes=100 * 1024 * 1024),
    )(
        A_x.reshape(1, M), c, w_mod,
        A_w_q.reshape(M * H, D), A_w_uk.reshape(DC * H, D),
        A_c_kv.reshape(SK, DC), A_w_uv.reshape(DC * H, D),
        A_w_o.reshape(H * D, M), B_w_gate, B_w_up, B_w_down,
    )
    return out.reshape(B, SQ, M)
```

```python
import functools

import jax
import jax.numpy as jnp
from jax import lax
import jax.experimental.pallas as pl
import jax.experimental.pallas.tpu as pltpu

_F32 = jnp.float32
_BF16 = jnp.bfloat16
_NT = (((1,), (1,)), ((), ()))
_LANES = 128
_CB = 512


def _layernorm(x, eps=1e-05):
    m = jnp.mean(x, axis=-1, keepdims=True)
    xc = x - m
    v = jnp.mean(xc * xc, axis=-1, keepdims=True)
    return xc / jnp.sqrt(v + eps)


def _row_splits(sizes):
    out, r0 = [], 0
    for n in sizes:
        out.append((r0, n))
        r0 += n
    return out


def _kernel(
    x_hbm, c_hbm, wmod_hbm, wq_hbm, wuk_hbm, ckv_hbm, wuv_hbm, wo_hbm,
    wg_hbm, wu_hbm, wd_hbm,
    o_ref,
    x_v, c_v, wmod_v, wq_v, wuk_v, ckv_v, wuv_v, wo_v, wg_v, wu_v, wd_v,
    e_v, s_v, ht_v, stage_s, sems, side_sems,
    *, H, D, M, DC, kv_chunks, tk, wd_mxu, wd_vpu, wu_side, service_at,
):
    copies = {}

    def add(name, src, dst, rows=None):
        if rows is not None:
            src = src.at[pl.ds(*rows)]
            dst = dst.at[pl.ds(*rows)]
        copies[name] = pltpu.make_async_copy(src, dst, sems.at[len(copies)])

    kv_rows = _row_splits(kv_chunks)
    wd_rows = _row_splits(tuple(wd_mxu) + tuple(wd_vpu))
    n_side = sum(wu_side)
    add("x", x_hbm, x_v)
    add("c", c_hbm, c_v)
    add("wmod", wmod_hbm, wmod_v)
    add("wq", wq_hbm, wq_v)
    add("wuk", wuk_hbm, wuk_v)
    for i, rows in enumerate(kv_rows):
        add(f"kv{i}", ckv_hbm, ckv_v, rows)
    add("wuv", wuv_hbm, wuv_v)
    add("wo", wo_hbm, wo_v)
    add("wu", wu_hbm, wu_v, (n_side, M - n_side))
    add("wg", wg_hbm, wg_v)
    for i, rows in enumerate(wd_rows):
        add(f"wd{i}", wd_hbm, wd_v, rows)

    to_smem, to_vmem = [], []
    for i, (r0, n) in enumerate(_row_splits(wu_side)):
        slot = stage_s.at[i % 2, pl.ds(0, n)]
        to_smem.append(pltpu.make_async_copy(
            wu_hbm.at[pl.ds(r0, n)], slot, side_sems.at[2 * i]))
        to_vmem.append(pltpu.make_async_copy(
            slot, wu_v.at[pl.ds(r0, n)], side_sems.at[2 * i + 1]))

    def service(pos):
        if pos not in service_at:
            return
        k = service_at.index(pos)
        if k < len(to_smem):
            to_smem[k].wait()
            to_vmem[k].start()
        if k >= 1:
            to_vmem[k - 1].wait()
            if k + 1 < len(to_smem):
                to_smem[k + 1].start()

    def wait(name):
        service(name)
        copies[name].wait()

    for cp in copies.values():
        cp.start()
    to_smem[0].start()
    to_smem[1].start()

    nblk = DC // _LANES
    ew = _LANES * H
    for j in range(ew // _CB):
        row = lax.broadcasted_iota(jnp.int32, (_LANES, _CB), 0)
        col = lax.broadcasted_iota(jnp.int32, (_LANES, _CB), 1) + j * _CB
        e_v[:, j * _CB:(j + 1) * _CB] = jnp.where(
            col // H == row, 1.0, 0.0).astype(_BF16)

    def head_mask(rows):
        row = lax.broadcasted_iota(jnp.int32, (rows, _CB), 0)
        col = lax.broadcasted_iota(jnp.int32, (rows, _CB), 1)
        return (col % H) == (row % H)

    def expand(a):
        a4 = jnp.concatenate(
            [jnp.broadcast_to(a[:, u * _LANES:(u + 1) * _LANES], (H, _LANES))
             for u in range(nblk)], axis=0).astype(_BF16)
        mask = head_mask(nblk * H)
        for j in range(ew // _CB):
            xj = jnp.dot(a4, e_v[:, j * _CB:(j + 1) * _CB],
                         preferred_element_type=_F32)
            xj = jnp.where(mask, xj, 0.0).astype(_BF16)
            for u in range(nblk):
                s_v[:, u * ew + j * _CB:u * ew + (j + 1) * _CB] = (
                    xj[u * H:(u + 1) * H, :])

    def per_head_matvec(w_v):
        parts = [
            jnp.dot(s_v[:, u * ew:(u + 1) * ew], w_v[u * ew:(u + 1) * ew, :],
                    preferred_element_type=_F32)
            for u in range(nblk)
        ]
        return functools.reduce(lambda a, b: a + b, parts)

    wait("x")
    wait("c")
    wait("wmod")
    cc = c_v[...].astype(_F32)
    silu_c = jnp.broadcast_to(cc * jax.nn.sigmoid(cc), (8, M)).astype(_BF16)
    mod = jnp.dot(silu_c, wmod_v[...], preferred_element_type=_F32)[0:1, :]
    sa, ca, ga, sb, cb, gb = (mod[:, i * M:(i + 1) * M] for i in range(6))
    x0 = x_v[...].astype(_F32)
    h1 = _layernorm(x0) * (1.0 + ca) + sa

    expand(h1)
    wait("wq")
    q = per_head_matvec(wq_v).astype(_BF16)

    wait("wuk")
    scale = float(D) ** -0.5
    mask = head_mask(H)
    for j in range(DC * H // _CB):
        rj = lax.dot_general(q, wuk_v[j * _CB:(j + 1) * _CB, :], _NT,
                             preferred_element_type=_F32)
        s_v[:, j * _CB:(j + 1) * _CB] = jnp.where(
            mask, rj * scale, 0.0).astype(_BF16)
    r4 = jnp.concatenate(
        [s_v[:, u * ew:(u + 1) * ew] for u in range(nblk)], axis=0)
    qa4 = lax.dot_general(r4, e_v[...], _NT,
                          preferred_element_type=_F32)
    qa = jnp.concatenate(
        [qa4[u * H:(u + 1) * H, :] for u in range(nblk)], axis=1
    ).astype(_BF16)

    def attn_step(start, carry):
        m, l, acc = carry
        kv = ckv_v[pl.ds(start, tk), :]
        s = lax.dot_general(qa, kv, _NT, preferred_element_type=_F32)
        m_new = jnp.maximum(m, jnp.max(s, axis=1, keepdims=True))
        alpha = jnp.exp(m - m_new)
        p = jnp.exp(s - m_new)
        l = l * alpha + jnp.sum(p, axis=1, keepdims=True)
        acc = acc * alpha + jnp.dot(p.astype(_BF16), kv,
                                    preferred_element_type=_F32)
        return m_new, l, acc

    carry = (jnp.full((H, 1), -jnp.inf, _F32), jnp.zeros((H, 1), _F32),
             jnp.zeros((H, DC), _F32))
    for i, (r0, n) in enumerate(kv_rows):
        wait(f"kv{i}")
        carry = lax.fori_loop(
            0, n // tk,
            lambda t, cr, r0=r0: attn_step(
                pl.multiple_of(r0 + t * tk, tk), cr),
            carry)
    _, l, acc = carry

    expand(acc / l)
    wait("wuv")
    ctx = per_head_matvec(wuv_v)

    row = lax.broadcasted_iota(jnp.int32, (H, D), 0)
    lhs = jnp.concatenate(
        [jnp.where(row == h, ctx, 0.0).astype(_BF16) for h in range(H)],
        axis=1)
    wait("wo")
    attn = jnp.sum(jnp.dot(lhs, wo_v[...], preferred_element_type=_F32),
                   axis=0, keepdims=True)
    x1 = x0 + ga * attn

    h2 = _layernorm(x1) * (1.0 + cb) + sb
    h2 = jnp.broadcast_to(h2, (8, M)).astype(_BF16)
    wait("wg")
    g = jnp.dot(h2, wg_v[...], preferred_element_type=_F32)
    g = jax.nn.gelu(g, approximate=True)
    wait("wu")
    u = jnp.dot(h2, wu_v[...], preferred_element_type=_F32)
    hf = (g * u).astype(_BF16)

    n_mxu = sum(wd_mxu)
    for j in range(sum(wd_vpu) // _LANES):
        c0 = n_mxu + j * _LANES
        blk = hf[0:1, c0:c0 + _LANES].astype(_F32)
        ht_v[j * _LANES:(j + 1) * _LANES, :] = jnp.broadcast_to(
            blk, (_LANES, _LANES)).T

    y = None
    for i, (r0, n) in enumerate(wd_rows[:len(wd_mxu)]):
        wait(f"wd{i}")
        part = jnp.dot(hf[:, r0:r0 + n], wd_v[r0:r0 + n, :],
                       preferred_element_type=_F32)
        y = part if y is None else part + y
    sub = lax.broadcasted_iota(jnp.int32, (8, M), 0)
    z = jnp.where(sub == 0, y, 0.0)
    for i in range(len(wd_mxu), len(wd_rows)):
        wait(f"wd{i}")
        r0, n = wd_rows[i]
        z_hi = None
        for r in range(r0, r0 + n, 16):
            w = wd_v[r:r + 16, :].astype(_F32)
            hcol = ht_v[r - n_mxu:r - n_mxu + 16, :]
            t = w * jnp.concatenate([hcol] * (M // _LANES), axis=1)
            z = z + t[0:8]
            z_hi = t[8:16] if z_hi is None else z_hi + t[8:16]
        z = z + z_hi
    y = jnp.sum(z, axis=0, keepdims=True)
    o_ref[...] = (x1 + gb * y).astype(o_ref.dtype)


@jax.jit
def pallas_adaLN_cond__compressed_kv_cla__glu_gated_geglu__decode_kernel(
    A_x: jax.Array,
    A_c_kv: jax.Array,
    A_w_q: jax.Array,
    A_w_uk: jax.Array,
    A_w_uv: jax.Array,
    A_w_o: jax.Array,
    B_x: jax.Array,
    B_w_gate: jax.Array,
    B_w_up: jax.Array,
    B_w_down: jax.Array,
    c: jax.Array,
    w_mod: jax.Array,
):
    del B_x
    B, SQ, M = A_x.shape
    _, SK, DC = A_c_kv.shape
    _, H, D = A_w_q.shape
    DF = B_w_gate.shape[1]
    assert B == 1 and SQ == 1 and M == DC

    kv_chunks = (SK // 8,) * 8
    tk = 2048
    wd_mxu = (1024, 384)
    wd_vpu = (256, 96, 32)
    wu_side = (128, 128, 128, 112)
    service_at = ("wuk", "kv1", "kv5", "wuv", "wu")
    assert sum(wd_mxu) + sum(wd_vpu) == DF and sum(wu_side) < M
    assert len(service_at) == len(wu_side) + 1
    n_dma = 9 + len(kv_chunks) + len(wd_mxu) + len(wd_vpu)

    kernel = functools.partial(
        _kernel, H=H, D=D, M=M, DC=DC, kv_chunks=kv_chunks, tk=tk,
        wd_mxu=wd_mxu, wd_vpu=wd_vpu, wu_side=wu_side, service_at=service_at)

    dt = A_x.dtype
    out = pl.pallas_call(
        kernel,
        out_shape=jax.ShapeDtypeStruct((1, M), dt),
        in_specs=[pl.BlockSpec(memory_space=pl.ANY)] * 11,
        out_specs=pl.BlockSpec(memory_space=pltpu.VMEM),
        scratch_shapes=[
            pltpu.VMEM((1, M), dt),
            pltpu.VMEM((1, M), dt),
            pltpu.VMEM((M, 6 * M), dt),
            pltpu.VMEM((M * H, D), dt),
            pltpu.VMEM((DC * H, D), dt),
            pltpu.VMEM((SK, DC), dt),
            pltpu.VMEM((DC * H, D), dt),
            pltpu.VMEM((H * D, M), dt),
            pltpu.VMEM((M, DF), dt),
            pltpu.VMEM((M, DF), dt),
            pltpu.VMEM((DF, M), dt),
            pltpu.VMEM((_LANES, _LANES * H), _BF16),
            pltpu.VMEM((H, DC * H), _BF16),
            pltpu.VMEM((sum(wd_vpu), _LANES), _F32),
            pltpu.SMEM((2, max(wu_side), DF), dt),
            pltpu.SemaphoreType.DMA((n_dma,)),
            pltpu.SemaphoreType.DMA((2 * len(wu_side),)),
        ],
        compiler_params=pltpu.CompilerParams(
            vmem_limit_bytes=100 * 1024 * 1024,
            disable_semaphore_checks=True),
    )(
        A_x.reshape(1, M), c, w_mod,
        A_w_q.reshape(M * H, D), A_w_uk.reshape(DC * H, D),
        A_c_kv.reshape(SK, DC), A_w_uv.reshape(DC * H, D),
        A_w_o.reshape(H * D, M), B_w_gate, B_w_up, B_w_down,
    )
    return out.reshape(B, SQ, M)
```

```python
import functools

import jax
import jax.numpy as jnp
from jax import lax
import jax.experimental.pallas as pl
import jax.experimental.pallas.tpu as pltpu

_F32 = jnp.float32
_BF16 = jnp.bfloat16
_NT = (((1,), (1,)), ((), ()))
_LANES = 128
_CB = 512


def _layernorm(x, eps=1e-05):
    m = jnp.mean(x, axis=-1, keepdims=True)
    xc = x - m
    v = jnp.mean(xc * xc, axis=-1, keepdims=True)
    return xc / jnp.sqrt(v + eps)


def _row_splits(sizes):
    out, r0 = [], 0
    for n in sizes:
        out.append((r0, n))
        r0 += n
    return out


def _kernel(
    x_hbm, c_hbm, wmod_hbm, wq_hbm, wuk_hbm, ckv_hbm, wuv_hbm, wo_hbm,
    wg_hbm, wu_hbm, wd_hbm,
    o_ref,
    x_v, c_v, wmod_v, wq_v, wuk_v, ckv_v, wuv_v, wo_v, wg_v, wu_v, wd_v,
    e_v, s_v, ht_v, stage_s, sems, side_sems,
    *, H, D, M, DC, kv_chunks, tk, n_mxu, wd_vpu, wu_side, service_at,
):
    copies = {}

    def add(name, src, dst, rows=None):
        if rows is not None:
            src = src.at[pl.ds(*rows)]
            dst = dst.at[pl.ds(*rows)]
        copies[name] = pltpu.make_async_copy(src, dst, sems.at[len(copies)])

    kv_rows = _row_splits(kv_chunks)
    wd_rows = _row_splits((n_mxu,) + tuple(wd_vpu))
    n_side = sum(wu_side)
    add("wmod", wmod_hbm, wmod_v)
    add("x", x_hbm, x_v)
    add("c", c_hbm, c_v)
    add("wq", wq_hbm, wq_v)
    add("wuk", wuk_hbm, wuk_v)
    for i, rows in enumerate(kv_rows):
        add(f"kv{i}", ckv_hbm, ckv_v, rows)
    add("wuv", wuv_hbm, wuv_v)
    add("wo", wo_hbm, wo_v)
    add("wu", wu_hbm, wu_v, (n_side, M - n_side))
    add("wg", wg_hbm, wg_v)
    for i, rows in enumerate(wd_rows):
        add(f"wd{i}", wd_hbm, wd_v, rows)

    to_smem, to_vmem = [], []
    for i, (r0, n) in enumerate(_row_splits(wu_side)):
        slot = stage_s.at[i % 2, pl.ds(0, n)]
        to_smem.append(pltpu.make_async_copy(
            wu_hbm.at[pl.ds(r0, n)], slot, side_sems.at[2 * i]))
        to_vmem.append(pltpu.make_async_copy(
            slot, wu_v.at[pl.ds(r0, n)], side_sems.at[2 * i + 1]))

    def service(pos):
        if pos not in service_at:
            return
        k = service_at.index(pos)
        if k < len(to_smem):
            to_smem[k].wait()
            to_vmem[k].start()
        if k >= 1:
            to_vmem[k - 1].wait()
            if k + 1 < len(to_smem):
                to_smem[k + 1].start()

    def wait(name):
        service(name)
        copies[name].wait()

    for cp in copies.values():
        cp.start()
    to_smem[0].start()
    to_smem[1].start()

    nblk = DC // _LANES
    ew = _LANES * H
    for j in range(ew // _CB):
        row = lax.broadcasted_iota(jnp.int32, (_LANES, _CB), 0)
        col = lax.broadcasted_iota(jnp.int32, (_LANES, _CB), 1) + j * _CB
        e_v[:, j * _CB:(j + 1) * _CB] = jnp.where(
            col // H == row, 1.0, 0.0).astype(_BF16)

    def head_mask(rows):
        row = lax.broadcasted_iota(jnp.int32, (rows, _CB), 0)
        col = lax.broadcasted_iota(jnp.int32, (rows, _CB), 1)
        return (col % H) == (row % H)

    def expand(a):
        a4 = jnp.concatenate(
            [jnp.broadcast_to(a[:, u * _LANES:(u + 1) * _LANES], (H, _LANES))
             for u in range(nblk)], axis=0).astype(_BF16)
        mask = head_mask(nblk * H)
        for j in range(ew // _CB):
            xj = jnp.dot(a4, e_v[:, j * _CB:(j + 1) * _CB],
                         preferred_element_type=_F32)
            xj = jnp.where(mask, xj, 0.0).astype(_BF16)
            for u in range(nblk):
                s_v[:, u * ew + j * _CB:u * ew + (j + 1) * _CB] = (
                    xj[u * H:(u + 1) * H, :])

    def per_head_matvec(w_v):
        parts = [
            jnp.dot(s_v[:, u * ew:(u + 1) * ew], w_v[u * ew:(u + 1) * ew, :],
                    preferred_element_type=_F32)
            for u in range(nblk)
        ]
        return functools.reduce(lambda a, b: a + b, parts)

    wait("wmod")
    wait("x")
    wait("c")
    cc = c_v[...].astype(_F32)
    silu_c = jnp.broadcast_to(cc * jax.nn.sigmoid(cc), (8, M)).astype(_BF16)
    mod = jnp.dot(silu_c, wmod_v[...], preferred_element_type=_F32)[0:1, :]
    sa, ca, ga, sb, cb, gb = (mod[:, i * M:(i + 1) * M] for i in range(6))
    x0 = x_v[...].astype(_F32)
    h1 = _layernorm(x0) * (1.0 + ca) + sa

    expand(h1)
    wait("wq")
    q = per_head_matvec(wq_v).astype(_BF16)

    wait("wuk")
    scale = float(D) ** -0.5
    mask = head_mask(H)
    for j in range(DC * H // _CB):
        rj = lax.dot_general(q, wuk_v[j * _CB:(j + 1) * _CB, :], _NT,
                             preferred_element_type=_F32)
        s_v[:, j * _CB:(j + 1) * _CB] = jnp.where(
            mask, rj * scale, 0.0).astype(_BF16)
    r4 = jnp.concatenate(
        [s_v[:, u * ew:(u + 1) * ew] for u in range(nblk)], axis=0)
    qa4 = lax.dot_general(r4, e_v[...], _NT,
                          preferred_element_type=_F32)
    qa = jnp.concatenate(
        [qa4[u * H:(u + 1) * H, :] for u in range(nblk)], axis=1
    ).astype(_BF16)

    def attn_step(start, carry):
        m, l, acc = carry
        kv = ckv_v[pl.ds(start, tk), :]
        s = lax.dot_general(qa, kv, _NT, preferred_element_type=_F32)
        m_new = jnp.maximum(m, jnp.max(s, axis=1, keepdims=True))
        alpha = jnp.exp(m - m_new)
        p = jnp.exp(s - m_new)
        l = l * alpha + jnp.sum(p, axis=1, keepdims=True)
        acc = acc * alpha + jnp.dot(p.astype(_BF16), kv,
                                    preferred_element_type=_F32)
        return m_new, l, acc

    carry = (jnp.full((H, 1), -jnp.inf, _F32), jnp.zeros((H, 1), _F32),
             jnp.zeros((H, DC), _F32))
    for i, (r0, n) in enumerate(kv_rows):
        wait(f"kv{i}")
        carry = lax.fori_loop(
            0, n // tk,
            lambda t, cr, r0=r0: attn_step(
                pl.multiple_of(r0 + t * tk, tk), cr),
            carry)
    _, l, acc = carry

    expand(acc / l)
    wait("wuv")
    ctx = per_head_matvec(wuv_v)

    row = lax.broadcasted_iota(jnp.int32, (H, D), 0)
    lhs = jnp.concatenate(
        [jnp.where(row == h, ctx, 0.0).astype(_BF16) for h in range(H)],
        axis=1)
    wait("wo")
    attn = jnp.sum(jnp.dot(lhs, wo_v[...], preferred_element_type=_F32),
                   axis=0, keepdims=True)
    x1 = x0 + ga * attn

    h2 = _layernorm(x1) * (1.0 + cb) + sb
    h2 = jnp.broadcast_to(h2, (8, M)).astype(_BF16)
    n_early = sum(wu_side[:-1])
    u = jnp.dot(h2[:, :n_early], wu_v[:n_early, :],
                preferred_element_type=_F32)
    wait("wg")
    g = jnp.dot(h2, wg_v[...], preferred_element_type=_F32)
    g = jax.nn.gelu(g, approximate=True)
    wait("wu")
    u = jnp.dot(h2[:, n_early:], wu_v[n_early:, :],
                preferred_element_type=_F32) + u
    hf = (g * u).astype(_BF16)

    wait("wd0")
    y = jnp.dot(hf[:, :n_mxu], wd_v[:n_mxu, :], preferred_element_type=_F32)
    for j in range(sum(wd_vpu) // _LANES):
        c0 = n_mxu + j * _LANES
        blk = hf[0:1, c0:c0 + _LANES].astype(_F32)
        ht_v[j * _LANES:(j + 1) * _LANES, :] = jnp.broadcast_to(
            blk, (_LANES, _LANES)).T
    sub = lax.broadcasted_iota(jnp.int32, (8, M), 0)
    z = jnp.where(sub == 0, y, 0.0)
    for i in range(1, len(wd_rows)):
        wait(f"wd{i}")
        r0, n = wd_rows[i]
        z_hi = None
        for r in range(r0, r0 + n, 16):
            w = wd_v[r:r + 16, :].astype(_F32)
            hcol = ht_v[r - n_mxu:r - n_mxu + 16, :]
            t = w * jnp.concatenate([hcol] * (M // _LANES), axis=1)
            z = z + t[0:8]
            z_hi = t[8:16] if z_hi is None else z_hi + t[8:16]
        z = z + z_hi
    y = jnp.sum(z, axis=0, keepdims=True)
    o_ref[...] = (x1 + gb * y).astype(o_ref.dtype)


@jax.jit
def pallas_adaLN_cond__compressed_kv_cla__glu_gated_geglu__decode_kernel(
    A_x: jax.Array,
    A_c_kv: jax.Array,
    A_w_q: jax.Array,
    A_w_uk: jax.Array,
    A_w_uv: jax.Array,
    A_w_o: jax.Array,
    B_x: jax.Array,
    B_w_gate: jax.Array,
    B_w_up: jax.Array,
    B_w_down: jax.Array,
    c: jax.Array,
    w_mod: jax.Array,
):
    del B_x
    B, SQ, M = A_x.shape
    _, SK, DC = A_c_kv.shape
    _, H, D = A_w_q.shape
    DF = B_w_gate.shape[1]
    assert B == 1 and SQ == 1 and M == DC

    kv_chunks = (SK // 8,) * 8
    tk = 2048
    n_mxu = 1024
    wd_vpu = (384, 256, 96, 32)
    wu_side = (128, 128, 128, 112)
    service_at = ("wuk", "kv1", "kv5", "wuv", "wu")
    assert n_mxu + sum(wd_vpu) == DF and sum(wu_side) < M
    assert len(service_at) == len(wu_side) + 1
    n_dma = 10 + len(kv_chunks) + len(wd_vpu)

    kernel = functools.partial(
        _kernel, H=H, D=D, M=M, DC=DC, kv_chunks=kv_chunks, tk=tk,
        n_mxu=n_mxu, wd_vpu=wd_vpu, wu_side=wu_side, service_at=service_at)

    dt = A_x.dtype
    out = pl.pallas_call(
        kernel,
        out_shape=jax.ShapeDtypeStruct((1, M), dt),
        in_specs=[pl.BlockSpec(memory_space=pl.ANY)] * 11,
        out_specs=pl.BlockSpec(memory_space=pltpu.VMEM),
        scratch_shapes=[
            pltpu.VMEM((1, M), dt),
            pltpu.VMEM((1, M), dt),
            pltpu.VMEM((M, 6 * M), dt),
            pltpu.VMEM((M * H, D), dt),
            pltpu.VMEM((DC * H, D), dt),
            pltpu.VMEM((SK, DC), dt),
            pltpu.VMEM((DC * H, D), dt),
            pltpu.VMEM((H * D, M), dt),
            pltpu.VMEM((M, DF), dt),
            pltpu.VMEM((M, DF), dt),
            pltpu.VMEM((DF, M), dt),
            pltpu.VMEM((_LANES, _LANES * H), _BF16),
            pltpu.VMEM((H, DC * H), _BF16),
            pltpu.VMEM((sum(wd_vpu), _LANES), _F32),
            pltpu.SMEM((2, max(wu_side), DF), dt),
            pltpu.SemaphoreType.DMA((n_dma,)),
            pltpu.SemaphoreType.DMA((2 * len(wu_side),)),
        ],
        compiler_params=pltpu.CompilerParams(
            vmem_limit_bytes=100 * 1024 * 1024,
            disable_semaphore_checks=True),
    )(
        A_x.reshape(1, M), c, w_mod,
        A_w_q.reshape(M * H, D), A_w_uk.reshape(DC * H, D),
        A_c_kv.reshape(SK, DC), A_w_uv.reshape(DC * H, D),
        A_w_o.reshape(H * D, M), B_w_gate, B_w_up, B_w_down,
    )
    return out.reshape(B, SQ, M)
```

```python
import functools

import jax
import jax.numpy as jnp
from jax import lax
import jax.experimental.pallas as pl
import jax.experimental.pallas.tpu as pltpu

_F32 = jnp.float32
_BF16 = jnp.bfloat16
_NT = (((1,), (1,)), ((), ()))
_LANES = 128
_CB = 512


def _layernorm(x, eps=1e-05):
    m = jnp.mean(x, axis=-1, keepdims=True)
    xc = x - m
    v = jnp.mean(xc * xc, axis=-1, keepdims=True)
    return xc / jnp.sqrt(v + eps)


def _row_splits(sizes):
    out, r0 = [], 0
    for n in sizes:
        out.append((r0, n))
        r0 += n
    return out


def _kernel(*refs, n_dma, **params):
    pl.run_scoped(
        functools.partial(_body, *refs, **params),
        pltpu.SemaphoreType.DMA((n_dma,)),
        pltpu.SemaphoreType.DMA((2 * len(params["wu_side"]),)),
    )


def _body(
    x_hbm, c_hbm, wmod_hbm, wq_hbm, wuk_hbm, ckv_hbm, wuv_hbm, wo_hbm,
    wg_hbm, wu_hbm, wd_hbm,
    o_ref,
    x_v, c_v, wmod_v, wq_v, wuk_v, ckv_v, wuv_v, wo_v, wg_v, wu_v, wd_v,
    e_v, s_v, ht_v, stage_s, sems, side_sems,
    *, H, D, M, DC, kv_chunks, tk, n_mxu, wd_vpu, wu_side, service_at,
):
    copies = {}

    def add(name, src, dst, rows=None):
        if rows is not None:
            src = src.at[pl.ds(*rows)]
            dst = dst.at[pl.ds(*rows)]
        copies[name] = pltpu.make_async_copy(src, dst, sems.at[len(copies)])

    kv_rows = _row_splits(kv_chunks)
    wd_rows = _row_splits((n_mxu,) + tuple(wd_vpu))
    n_side = sum(wu_side)
    add("wmod", wmod_hbm, wmod_v)
    add("x", x_hbm, x_v)
    add("c", c_hbm, c_v)
    add("wq", wq_hbm, wq_v)
    add("wuk", wuk_hbm, wuk_v)
    for i, rows in enumerate(kv_rows):
        add(f"kv{i}", ckv_hbm, ckv_v, rows)
    add("wuv", wuv_hbm, wuv_v)
    add("wo", wo_hbm, wo_v)
    add("wu", wu_hbm, wu_v, (n_side, M - n_side))
    add("wg", wg_hbm, wg_v)
    for i, rows in enumerate(wd_rows):
        add(f"wd{i}", wd_hbm, wd_v, rows)

    to_smem, to_vmem = [], []
    for i, (r0, n) in enumerate(_row_splits(wu_side)):
        slot = stage_s.at[i % 2, pl.ds(0, n)]
        to_smem.append(pltpu.make_async_copy(
            wu_hbm.at[pl.ds(r0, n)], slot, side_sems.at[2 * i]))
        to_vmem.append(pltpu.make_async_copy(
            slot, wu_v.at[pl.ds(r0, n)], side_sems.at[2 * i + 1]))

    def service(pos):
        if pos not in service_at:
            return
        k = service_at.index(pos)
        if k < len(to_smem):
            to_smem[k].wait()
            to_vmem[k].start()
        if k >= 1:
            to_vmem[k - 1].wait()
            if k + 1 < len(to_smem):
                to_smem[k + 1].start()

    def wait(name):
        service(name)
        copies[name].wait()

    for cp in copies.values():
        cp.start()
    to_smem[0].start()
    to_smem[1].start()

    nblk = DC // _LANES
    ew = _LANES * H
    for j in range(ew // _CB):
        row = lax.broadcasted_iota(jnp.int32, (_LANES, _CB), 0)
        col = lax.broadcasted_iota(jnp.int32, (_LANES, _CB), 1) + j * _CB
        e_v[:, j * _CB:(j + 1) * _CB] = jnp.where(
            col // H == row, 1.0, 0.0).astype(_BF16)

    def head_mask(rows):
        row = lax.broadcasted_iota(jnp.int32, (rows, _CB), 0)
        col = lax.broadcasted_iota(jnp.int32, (rows, _CB), 1)
        return (col % H) == (row % H)

    def expand(a):
        a4 = jnp.concatenate(
            [jnp.broadcast_to(a[:, u * _LANES:(u + 1) * _LANES], (H, _LANES))
             for u in range(nblk)], axis=0).astype(_BF16)
        mask = head_mask(nblk * H)
        for j in range(ew // _CB):
            xj = jnp.dot(a4, e_v[:, j * _CB:(j + 1) * _CB],
                         preferred_element_type=_F32)
            xj = jnp.where(mask, xj, 0.0).astype(_BF16)
            for u in range(nblk):
                s_v[:, u * ew + j * _CB:u * ew + (j + 1) * _CB] = (
                    xj[u * H:(u + 1) * H, :])

    def per_head_matvec(w_v):
        parts = [
            jnp.dot(s_v[:, u * ew:(u + 1) * ew], w_v[u * ew:(u + 1) * ew, :],
                    preferred_element_type=_F32)
            for u in range(nblk)
        ]
        return functools.reduce(lambda a, b: a + b, parts)

    wait("wmod")
    wait("x")
    wait("c")
    cc = c_v[...].astype(_F32)
    silu_c = jnp.broadcast_to(cc * jax.nn.sigmoid(cc), (8, M)).astype(_BF16)
    mod = jnp.dot(silu_c, wmod_v[...], preferred_element_type=_F32)[0:1, :]
    sa, ca, ga, sb, cb, gb = (mod[:, i * M:(i + 1) * M] for i in range(6))
    x0 = x_v[...].astype(_F32)
    h1 = _layernorm(x0) * (1.0 + ca) + sa

    expand(h1)
    wait("wq")
    q = per_head_matvec(wq_v).astype(_BF16)

    wait("wuk")
    scale = float(D) ** -0.5
    mask = head_mask(H)
    for j in range(DC * H // _CB):
        rj = lax.dot_general(q, wuk_v[j * _CB:(j + 1) * _CB, :], _NT,
                             preferred_element_type=_F32)
        s_v[:, j * _CB:(j + 1) * _CB] = jnp.where(
            mask, rj * scale, 0.0).astype(_BF16)
    r4 = jnp.concatenate(
        [s_v[:, u * ew:(u + 1) * ew] for u in range(nblk)], axis=0)
    qa4 = lax.dot_general(r4, e_v[...], _NT,
                          preferred_element_type=_F32)
    qa = jnp.concatenate(
        [qa4[u * H:(u + 1) * H, :] for u in range(nblk)], axis=1
    ).astype(_BF16)

    def attn_step(start, carry):
        m, l, acc = carry
        kv = ckv_v[pl.ds(start, tk), :]
        s = lax.dot_general(qa, kv, _NT, preferred_element_type=_F32)
        m_new = jnp.maximum(m, jnp.max(s, axis=1, keepdims=True))
        alpha = jnp.exp(m - m_new)
        p = jnp.exp(s - m_new)
        l = l * alpha + jnp.sum(p, axis=1, keepdims=True)
        acc = acc * alpha + jnp.dot(p.astype(_BF16), kv,
                                    preferred_element_type=_F32)
        return m_new, l, acc

    carry = (jnp.full((H, 1), -jnp.inf, _F32), jnp.zeros((H, 1), _F32),
             jnp.zeros((H, DC), _F32))
    for i, (r0, n) in enumerate(kv_rows):
        wait(f"kv{i}")
        carry = lax.fori_loop(
            0, n // tk,
            lambda t, cr, r0=r0: attn_step(
                pl.multiple_of(r0 + t * tk, tk), cr),
            carry)
    _, l, acc = carry

    expand(acc / l)
    wait("wuv")
    ctx = per_head_matvec(wuv_v)

    row = lax.broadcasted_iota(jnp.int32, (H, D), 0)
    lhs = jnp.concatenate(
        [jnp.where(row == h, ctx, 0.0).astype(_BF16) for h in range(H)],
        axis=1)
    wait("wo")
    attn = jnp.sum(jnp.dot(lhs, wo_v[...], preferred_element_type=_F32),
                   axis=0, keepdims=True)
    x1 = x0 + ga * attn

    h2 = _layernorm(x1) * (1.0 + cb) + sb
    h2 = jnp.broadcast_to(h2, (8, M)).astype(_BF16)
    n_early = sum(wu_side[:-1])
    u = jnp.dot(h2[:, :n_early], wu_v[:n_early, :],
                preferred_element_type=_F32)
    wait("wg")
    g = jnp.dot(h2, wg_v[...], preferred_element_type=_F32)
    g = jax.nn.gelu(g, approximate=True)
    wait("wu")
    u = jnp.dot(h2[:, n_early:], wu_v[n_early:, :],
                preferred_element_type=_F32) + u
    hf = (g * u).astype(_BF16)

    wait("wd0")
    y = jnp.dot(hf[:, :n_mxu], wd_v[:n_mxu, :], preferred_element_type=_F32)
    for j in range(sum(wd_vpu) // _LANES):
        c0 = n_mxu + j * _LANES
        blk = hf[0:1, c0:c0 + _LANES].astype(_F32)
        ht_v[j * _LANES:(j + 1) * _LANES, :] = jnp.broadcast_to(
            blk, (_LANES, _LANES)).T
    sub = lax.broadcasted_iota(jnp.int32, (8, M), 0)
    z = jnp.where(sub == 0, y, 0.0)
    for i in range(1, len(wd_rows)):
        wait(f"wd{i}")
        r0, n = wd_rows[i]
        z_hi = None
        for r in range(r0, r0 + n, 16):
            w = wd_v[r:r + 16, :].astype(_F32)
            hcol = ht_v[r - n_mxu:r - n_mxu + 16, :]
            t = w * jnp.concatenate([hcol] * (M // _LANES), axis=1)
            z = z + t[0:8]
            z_hi = t[8:16] if z_hi is None else z_hi + t[8:16]
        z = z + z_hi
    y = jnp.sum(z, axis=0, keepdims=True)
    o_ref[...] = (x1 + gb * y).astype(o_ref.dtype)


@jax.jit
def pallas_adaLN_cond__compressed_kv_cla__glu_gated_geglu__decode_kernel(
    A_x: jax.Array,
    A_c_kv: jax.Array,
    A_w_q: jax.Array,
    A_w_uk: jax.Array,
    A_w_uv: jax.Array,
    A_w_o: jax.Array,
    B_x: jax.Array,
    B_w_gate: jax.Array,
    B_w_up: jax.Array,
    B_w_down: jax.Array,
    c: jax.Array,
    w_mod: jax.Array,
):
    del B_x
    B, SQ, M = A_x.shape
    _, SK, DC = A_c_kv.shape
    _, H, D = A_w_q.shape
    DF = B_w_gate.shape[1]
    assert B == 1 and SQ == 1 and M == DC

    kv_chunks = (SK // 8,) * 8
    tk = 2048
    n_mxu = 1024
    wd_vpu = (384, 256, 96, 32)
    wu_side = (128, 128, 128, 112)
    service_at = ("wuk", "kv1", "kv5", "wuv", "wu")
    assert n_mxu + sum(wd_vpu) == DF and sum(wu_side) < M
    assert len(service_at) == len(wu_side) + 1
    n_dma = 10 + len(kv_chunks) + len(wd_vpu)

    kernel = functools.partial(
        _kernel, n_dma=n_dma, H=H, D=D, M=M, DC=DC, kv_chunks=kv_chunks, tk=tk,
        n_mxu=n_mxu, wd_vpu=wd_vpu, wu_side=wu_side, service_at=service_at)

    dt = A_x.dtype
    out = pl.pallas_call(
        kernel,
        out_shape=jax.ShapeDtypeStruct((1, M), dt),
        in_specs=[pl.BlockSpec(memory_space=pl.ANY)] * 11,
        out_specs=pl.BlockSpec(memory_space=pltpu.VMEM),
        scratch_shapes=[
            pltpu.VMEM((1, M), dt),
            pltpu.VMEM((1, M), dt),
            pltpu.VMEM((M, 6 * M), dt),
            pltpu.VMEM((M * H, D), dt),
            pltpu.VMEM((DC * H, D), dt),
            pltpu.VMEM((SK, DC), dt),
            pltpu.VMEM((DC * H, D), dt),
            pltpu.VMEM((H * D, M), dt),
            pltpu.VMEM((M, DF), dt),
            pltpu.VMEM((M, DF), dt),
            pltpu.VMEM((DF, M), dt),
            pltpu.VMEM((_LANES, _LANES * H), _BF16),
            pltpu.VMEM((H, DC * H), _BF16),
            pltpu.VMEM((sum(wd_vpu), _LANES), _F32),
            pltpu.SMEM((2, max(wu_side), DF), dt),
        ],
        compiler_params=pltpu.CompilerParams(
            vmem_limit_bytes=100 * 1024 * 1024),
    )(
        A_x.reshape(1, M), c, w_mod,
        A_w_q.reshape(M * H, D), A_w_uk.reshape(DC * H, D),
        A_c_kv.reshape(SK, DC), A_w_uv.reshape(DC * H, D),
        A_w_o.reshape(H * D, M), B_w_gate, B_w_up, B_w_down,
    )
    return out.reshape(B, SQ, M)
```

```python
import functools

import jax
import jax.numpy as jnp
from jax import lax
import jax.experimental.pallas as pl
import jax.experimental.pallas.tpu as pltpu

_F32 = jnp.float32
_BF16 = jnp.bfloat16
_NT = (((1,), (1,)), ((), ()))
_LANES = 128
_CB = 512


def _layernorm(x, eps=1e-05):
    m = jnp.mean(x, axis=-1, keepdims=True)
    xc = x - m
    v = jnp.mean(xc * xc, axis=-1, keepdims=True)
    return xc / jnp.sqrt(v + eps)


def _row_splits(sizes):
    out, r0 = [], 0
    for n in sizes:
        out.append((r0, n))
        r0 += n
    return out


def _kernel(*refs, n_sem, **params):
    pl.run_scoped(
        functools.partial(_body, *refs, **params),
        pltpu.SemaphoreType.DMA((n_sem,)),
    )


def _body(
    x_hbm, c_hbm, wmod_hbm, wq_hbm, wuk_hbm, ckv_hbm, wuv_hbm, wo_hbm,
    wg_hbm, wu_hbm, wd_hbm,
    o_ref,
    x_v, c_v, wmod_v, wq_v, wuk_v, ckv_v, wuv_v, wo_v, wg_v, wu_v, wd_v,
    e_v, s_v, ht_v, stage_s, sems,
    *, H, D, M, DC, n_mxu, wd_vpu, wu_side, service_at, issue_plan, kv_early,
):
    n_kv = ckv_v.shape[0]
    tk = ckv_v.shape[1] * ckv_v.shape[2]
    starts, waits, sem_ids = {}, {}, {}

    def sem(name):
        return sems.at[sem_ids.setdefault(name, len(sem_ids))]

    def add(name, src, dst, rows=None):
        if rows is not None:
            src = src.at[pl.ds(*rows)]
            dst = dst.at[pl.ds(*rows)]
        waits[name] = pltpu.make_async_copy(src, dst, sem(name))
        starts[name] = [waits[name]]

    def add_strided(name, src, dst):
        starts[name] = [
            pltpu.make_async_copy(src.at[:, i], dst.at[:, i], sem(name))
            for i in range(src.shape[1])]
        waits[name] = pltpu.make_async_copy(dst, dst, sem(name))

    def kv_copy(i):
        return pltpu.make_async_copy(ckv_hbm.at[:, i], ckv_v.at[i], sems.at[i])

    for i in range(n_kv):
        sem(f"kv{i}")
    wd_rows = _row_splits((n_mxu,) + tuple(wd_vpu))
    n_side = sum(wu_side)
    for i in range(kv_early):
        starts[f"kv{i}"] = [kv_copy(i)]
    add_strided("wmod", wmod_hbm, wmod_v)
    add("x", x_hbm, x_v)
    add("c", c_hbm, c_v)
    add_strided("wq", wq_hbm, wq_v)
    add_strided("wuk", wuk_hbm, wuk_v)
    for i in range(kv_early, n_kv):
        starts[f"kv{i}"] = [kv_copy(i)]
    add_strided("wuv", wuv_hbm, wuv_v)
    add("wo", wo_hbm, wo_v)
    add("wu", wu_hbm, wu_v, (n_side, M - n_side))
    add("wg", wg_hbm, wg_v)
    for i, rows in enumerate(wd_rows):
        add(f"wd{i}", wd_hbm, wd_v, rows)

    names = list(starts)
    cuts = sorted((names.index(n), g) for g, n in issue_plan.items())
    assert cuts[0] == (0, 0)
    groups = {g: names[a:b] for (a, g), (b, _) in
              zip(cuts, cuts[1:] + [(len(names), None)])}

    def issue(g):
        for name in groups.pop(g, ()):
            for cp in starts[name]:
                cp.start()

    to_smem, to_vmem = [], []
    for i, (r0, n) in enumerate(_row_splits(wu_side)):
        slot = stage_s.at[i % 2, pl.ds(0, n)]
        to_smem.append(pltpu.make_async_copy(
            wu_hbm.at[pl.ds(r0, n)], slot, sem(f"to_smem{i}")))
        to_vmem.append(pltpu.make_async_copy(
            slot, wu_v.at[pl.ds(r0, n)], sem(f"to_vmem{i}")))

    def service(pos):
        for k in range(len(service_at)):
            if service_at[k] != pos:
                continue
            if k < len(to_smem):
                to_smem[k].wait()
                to_vmem[k].start()
            if k >= 1:
                to_vmem[k - 1].wait()
                if k + 1 < len(to_smem):
                    to_smem[k + 1].start()
            issue(k + 1)

    def wait(name):
        service(name)
        waits[name].wait()

    to_smem[0].start()
    to_smem[1].start()
    issue(0)

    nblk = DC // _LANES
    ew = _LANES * H
    for j in range(ew // _CB):
        row = lax.broadcasted_iota(jnp.int32, (_LANES, _CB), 0)
        col = lax.broadcasted_iota(jnp.int32, (_LANES, _CB), 1) + j * _CB
        e_v[:, j * _CB:(j + 1) * _CB] = jnp.where(
            col // H == row, 1.0, 0.0).astype(_BF16)

    def head_mask(rows):
        row = lax.broadcasted_iota(jnp.int32, (rows, _CB), 0)
        col = lax.broadcasted_iota(jnp.int32, (rows, _CB), 1)
        return (col % H) == (row % H)

    def expand(a):
        a4 = jnp.concatenate(
            [jnp.broadcast_to(a[:, u * _LANES:(u + 1) * _LANES], (H, _LANES))
             for u in range(nblk)], axis=0).astype(_BF16)
        mask = head_mask(nblk * H)
        for j in range(ew // _CB):
            xj = jnp.dot(a4, e_v[:, j * _CB:(j + 1) * _CB],
                         preferred_element_type=_F32)
            xj = jnp.where(mask, xj, 0.0).astype(_BF16)
            for u in range(nblk):
                s_v[:, u * ew + j * _CB:u * ew + (j + 1) * _CB] = (
                    xj[u * H:(u + 1) * H, :])

    def rows_of(w_v, r0, n):
        _, nb, p, cols = w_v.shape
        if r0 % (nb * p) == 0 and n % (nb * p) == 0:
            blk = w_v[r0 // (nb * p):(r0 + n) // (nb * p)]
        else:
            a, b = divmod(r0, nb * p)
            assert b % p == 0 and n % p == 0 and b + n <= nb * p
            blk = w_v[a, b // p:(b + n) // p]
        return blk.reshape(n, cols)

    def per_head_matvec(w_v):
        parts = [
            jnp.dot(s_v[:, u * ew:(u + 1) * ew], rows_of(w_v, u * ew, ew),
                    preferred_element_type=_F32)
            for u in range(nblk)
        ]
        return functools.reduce(lambda a, b: a + b, parts)

    wait("wmod")
    wait("x")
    wait("c")
    cc = c_v[...].astype(_F32)
    silu_c = jnp.broadcast_to(cc * jax.nn.sigmoid(cc), (8, M)).astype(_BF16)
    mod = jnp.dot(silu_c, rows_of(wmod_v, 0, M),
                  preferred_element_type=_F32)[0:1, :]
    sa, ca, ga, sb, cb, gb = (mod[:, i * M:(i + 1) * M] for i in range(6))
    x0 = x_v[...].astype(_F32)
    h1 = _layernorm(x0) * (1.0 + ca) + sa

    expand(h1)
    wait("wq")
    q = per_head_matvec(wq_v).astype(_BF16)

    wait("wuk")
    scale = float(D) ** -0.5
    mask = head_mask(H)
    for j in range(DC * H // _CB):
        rj = lax.dot_general(q, rows_of(wuk_v, j * _CB, _CB), _NT,
                             preferred_element_type=_F32)
        s_v[:, j * _CB:(j + 1) * _CB] = jnp.where(
            mask, rj * scale, 0.0).astype(_BF16)
    r4 = jnp.concatenate(
        [s_v[:, u * ew:(u + 1) * ew] for u in range(nblk)], axis=0)
    qa4 = lax.dot_general(r4, e_v[...], _NT,
                          preferred_element_type=_F32)
    qa = jnp.concatenate(
        [qa4[u * H:(u + 1) * H, :] for u in range(nblk)], axis=1
    ).astype(_BF16)

    def attn_step(i, carry):
        m, l, acc = carry
        kv_copy(i).wait()
        kv = ckv_v[i].reshape(tk, DC)
        s = lax.dot_general(qa, kv, _NT, preferred_element_type=_F32)
        m_new = jnp.maximum(m, jnp.max(s, axis=1, keepdims=True))
        alpha = jnp.exp(m - m_new)
        p = jnp.exp(s - m_new)
        l = l * alpha + jnp.sum(p, axis=1, keepdims=True)
        acc = acc * alpha + jnp.dot(p.astype(_BF16), kv,
                                    preferred_element_type=_F32)
        return m_new, l, acc

    carry = (jnp.full((H, 1), -jnp.inf, _F32), jnp.zeros((H, 1), _F32),
             jnp.zeros((H, DC), _F32))
    segs = [0] + [i for i in range(1, n_kv) if f"kv{i}" in service_at] + [n_kv]
    for lo, hi in zip(segs[:-1], segs[1:]):
        service(f"kv{lo}")
        carry = lax.fori_loop(lo, hi, attn_step, carry)
    _, l, acc = carry

    expand(acc / l)
    wait("wuv")
    ctx = per_head_matvec(wuv_v)

    row = lax.broadcasted_iota(jnp.int32, (H, D), 0)
    lhs = jnp.concatenate(
        [jnp.where(row == h, ctx, 0.0).astype(_BF16) for h in range(H)],
        axis=1)
    wait("wo")
    attn = jnp.sum(jnp.dot(lhs, wo_v[...], preferred_element_type=_F32),
                   axis=0, keepdims=True)
    x1 = x0 + ga * attn

    h2 = _layernorm(x1) * (1.0 + cb) + sb
    h2 = jnp.broadcast_to(h2, (8, M)).astype(_BF16)
    n_early = sum(wu_side[:-1]) // _LANES * _LANES
    u = jnp.dot(h2[:, :n_early], wu_v[:n_early, :],
                preferred_element_type=_F32)
    wait("wg")
    g = jnp.dot(h2, wg_v[...], preferred_element_type=_F32)
    g = jax.nn.gelu(g, approximate=True)
    wait("wu")
    u = jnp.dot(h2[:, n_early:], wu_v[n_early:, :],
                preferred_element_type=_F32) + u
    hf = (g * u).astype(_BF16)

    wait("wd0")
    y = jnp.dot(hf[:, :n_mxu], wd_v[:n_mxu, :], preferred_element_type=_F32)
    for j in range(sum(wd_vpu) // _LANES):
        c0 = n_mxu + j * _LANES
        blk = hf[0:1, c0:c0 + _LANES].astype(_F32)
        ht_v[j * _LANES:(j + 1) * _LANES, :] = jnp.broadcast_to(
            blk, (_LANES, _LANES)).T
    sub = lax.broadcasted_iota(jnp.int32, (8, M), 0)
    z = jnp.where(sub == 0, y, 0.0)
    for i in range(1, len(wd_rows)):
        wait(f"wd{i}")
        r0, n = wd_rows[i]
        z_hi = None
        for r in range(r0, r0 + n, 16):
            w = wd_v[r:r + 16, :].astype(_F32)
            hcol = ht_v[r - n_mxu:r - n_mxu + 16, :]
            t = w * jnp.concatenate([hcol] * (M // _LANES), axis=1)
            z = z + t[0:8]
            z_hi = t[8:16] if z_hi is None else z_hi + t[8:16]
        z = z + z_hi
    assert not groups
    y = jnp.sum(z, axis=0, keepdims=True)
    o_ref[...] = (x1 + gb * y).astype(o_ref.dtype)


@jax.jit
def pallas_adaLN_cond__compressed_kv_cla__glu_gated_geglu__decode_kernel(
    A_x: jax.Array,
    A_c_kv: jax.Array,
    A_w_q: jax.Array,
    A_w_uk: jax.Array,
    A_w_uv: jax.Array,
    A_w_o: jax.Array,
    B_x: jax.Array,
    B_w_gate: jax.Array,
    B_w_up: jax.Array,
    B_w_down: jax.Array,
    c: jax.Array,
    w_mod: jax.Array,
):
    del B_x
    B, SQ, M = A_x.shape
    _, SK, DC = A_c_kv.shape
    _, H, D = A_w_q.shape
    DF = B_w_gate.shape[1]
    assert B == 1 and SQ == 1 and M == DC

    n_kv, kv_piece = 16, 32
    kv_shape = (SK // (n_kv * kv_piece), n_kv, kv_piece, DC)
    head_shape = (8, 16, M * H // 128, D)
    mod_shape = (4, M // 64, 16, 6 * M)
    n_mxu = 1024
    wd_vpu = (384, 256, 96, 32)
    wu_side = (32, 64, 96, 128, 128, 48)
    service_at = ("wmod", "wmod", "wuk", "kv7", "kv14", "wo", "wu")
    issue_plan = {0: "kv0", 2: "wq", 3: "kv4", 4: "wuv", 5: "wo"}
    assert n_mxu + sum(wd_vpu) == DF and sum(wu_side) < M
    assert len(service_at) == len(wu_side) + 1
    n_sem = 10 + n_kv + len(wd_vpu) + 2 * len(wu_side)

    kernel = functools.partial(
        _kernel, n_sem=n_sem, H=H, D=D, M=M, DC=DC, n_mxu=n_mxu, wd_vpu=wd_vpu,
        wu_side=wu_side, service_at=service_at, issue_plan=issue_plan,
        kv_early=4)

    dt = A_x.dtype
    out = pl.pallas_call(
        kernel,
        out_shape=jax.ShapeDtypeStruct((1, M), dt),
        in_specs=[pl.BlockSpec(memory_space=pl.ANY)] * 11,
        out_specs=pl.BlockSpec(memory_space=pltpu.VMEM),
        scratch_shapes=[
            pltpu.VMEM((1, M), dt),
            pltpu.VMEM((1, M), dt),
            pltpu.VMEM(mod_shape, dt),
            pltpu.VMEM(head_shape, dt),
            pltpu.VMEM(head_shape, dt),
            pltpu.VMEM((n_kv, kv_shape[0], kv_piece, DC), dt),
            pltpu.VMEM(head_shape, dt),
            pltpu.VMEM((H * D, M), dt),
            pltpu.VMEM((M, DF), dt),
            pltpu.VMEM((M, DF), dt),
            pltpu.VMEM((DF, M), dt),
            pltpu.VMEM((_LANES, _LANES * H), _BF16),
            pltpu.VMEM((H, DC * H), _BF16),
            pltpu.VMEM((sum(wd_vpu), _LANES), _F32),
            pltpu.SMEM((2, max(wu_side), DF), dt),
        ],
        compiler_params=pltpu.CompilerParams(
            vmem_limit_bytes=100 * 1024 * 1024),
    )(
        A_x.reshape(1, M), c, w_mod.reshape(mod_shape),
        A_w_q.reshape(head_shape), A_w_uk.reshape(head_shape),
        A_c_kv.reshape(kv_shape), A_w_uv.reshape(head_shape),
        A_w_o.reshape(H * D, M), B_w_gate, B_w_up, B_w_down,
    )
    return out.reshape(B, SQ, M)
```

```python
import functools

import jax
import jax.numpy as jnp
from jax import lax
import jax.experimental.pallas as pl
import jax.experimental.pallas.tpu as pltpu

_F32 = jnp.float32
_BF16 = jnp.bfloat16
_NT = (((1,), (1,)), ((), ()))
_LANES = 128
_CB = 512
_BT = 32


def _layernorm(x, eps=1e-05):
    m = jnp.mean(x, axis=-1, keepdims=True)
    xc = x - m
    v = jnp.mean(xc * xc, axis=-1, keepdims=True)
    return xc / jnp.sqrt(v + eps)


def _row_splits(sizes):
    out, r0 = [], 0
    for n in sizes:
        out.append((r0, n))
        r0 += n
    return out


def _tiles(x, groups):
    x = x.reshape(-1, 8, x.shape[-1] // _LANES, _LANES).transpose(0, 2, 1, 3)
    return x.reshape(groups, -1, 8, _LANES)


def _untile(t, ncol):
    t = t.reshape(-1, ncol, 8, _LANES)
    cols = [t[:, j].reshape(-1, _LANES) for j in range(ncol)]
    return jnp.concatenate(cols, axis=1)


def _kernel(*refs, n_sem, **params):
    pl.run_scoped(
        functools.partial(_body, *refs, **params),
        pltpu.SemaphoreType.DMA((n_sem,)),
    )


def _body(
    x_hbm, c_hbm, wmod_hbm, wq_hbm, wuk_hbm, ckv_hbm, wuv_hbm, wo_hbm,
    wg_hbm, wu_hbm, wd_hbm,
    o_ref,
    x_v, c_v, wmod_v, wq_v, wuk_v, ckv_v, wuv_v, wo_v, wg_v, wu_v, wd_v,
    e_v, s_v, ht_v, wu_s, wd_s, sems,
    *, H, D, M, DC, wd_parts, wd_side, wu_side, order, plan, first_blk,
):
    starts, waits, sem_ids = {}, {}, {}

    def sem(name):
        return sems.at[sem_ids.setdefault(name, len(sem_ids))]

    def add(name, src, dst, rows=None):
        if rows is not None:
            src = src.at[pl.ds(*rows)]
            dst = dst.at[pl.ds(*rows)]
        starts[name] = [pltpu.make_async_copy(src, dst, sem(name))]
        waits[name] = starts[name]

    def add_blocks(name, src, dst):
        nt = src.shape[1]
        cuts = sorted({0, nt, *range(first_blk[name], nt, _BT)})
        starts[name] = [
            pltpu.make_async_copy(src.at[:, pl.ds(a, b - a)],
                                  dst.at[:, pl.ds(a, b - a)], sem(name))
            for a, b in zip(cuts[:-1], cuts[1:])]
        waits[name] = [pltpu.make_async_copy(dst, dst, sem(name))]

    nblk = DC // _LANES
    kv_t = ckv_v.shape[1]
    n_kv = kv_t // _BT
    kv_rot = first_blk["kv"] // nblk * nblk

    def kv_tiles(t0, n, s):
        return pltpu.make_async_copy(
            ckv_hbm.at[:, pl.ds(t0, n)],
            ckv_v.at[:, pl.ds((t0 - kv_rot) % kv_t, n)], s)

    def kv_block(i):
        return pltpu.make_async_copy(
            ckv_hbm.at[:, pl.ds(first_blk["kv"] + _BT * i, _BT)],
            ckv_v.at[:, pl.ds(first_blk["kv"] - kv_rot + _BT * i, _BT)],
            sems.at[i])

    for i in range(n_kv - 1):
        sem(f"kv{i}")
        starts[f"kv{i}"] = [kv_block(i)]
    kv_last = f"kv{n_kv - 1}"
    tail0 = first_blk["kv"] + _BT * (n_kv - 1)
    starts[kv_last] = waits[kv_last] = [
        kv_tiles(tail0, kv_t - tail0, sem(kv_last)),
        kv_tiles(0, kv_rot, sem(kv_last))]
    starts["kvh"] = waits["kvh"] = [
        kv_tiles(kv_rot, first_blk["kv"] - kv_rot, sem("kvh"))]

    wd_rows = _row_splits(wd_parts)
    n_side = sum(wu_side)
    add_blocks("wmod", wmod_hbm, wmod_v)
    add("x", x_hbm, x_v)
    add("c", c_hbm, c_v)
    add_blocks("wq", wq_hbm, wq_v)
    add_blocks("wuk", wuk_hbm, wuk_v)
    add_blocks("wuv", wuv_hbm, wuv_v)
    add_blocks("wo", wo_hbm, wo_v)
    add("wu", wu_hbm, wu_v, (n_side, M - n_side))
    add("wg", wg_hbm, wg_v)
    for i, rows in enumerate(wd_rows):
        if i not in wd_side:
            add(f"wd{i}", wd_hbm, wd_v, rows)

    groups = [g.split() for g in order.split("|")]
    assert sorted(sum(groups, [])) == sorted(starts)

    def issue():
        for name in groups.pop(0):
            for cp in starts[name]:
                cp.start()

    to_smem, to_vmem = [], []

    def add_side(src, stage, dst, rows):
        k = len(to_smem)
        to_smem.append(pltpu.make_async_copy(
            src.at[pl.ds(*rows)], stage, sem(f"to_smem{k}")))
        to_vmem.append(pltpu.make_async_copy(
            stage, dst.at[pl.ds(*rows)], sem(f"to_vmem{k}")))

    n_slot = wu_s.shape[0]
    for k, rows in enumerate(_row_splits(wu_side)):
        add_side(wu_hbm, wu_s.at[k % n_slot, pl.ds(0, rows[1])], wu_v, rows)
    staged = _row_splits([wd_parts[i] for i in wd_side])
    for i, rows in zip(wd_side, staged):
        add_side(wd_hbm, wd_s.at[pl.ds(*rows)], wd_v, wd_rows[i])
        waits[f"wd{i}"] = [to_vmem[-1]]
    waits["wu"] = to_vmem[len(wu_side) - n_slot:len(wu_side)] + waits["wu"]

    def fetch(k):
        if n_slot <= k < len(wu_side):
            to_vmem[k - n_slot].wait()
        if k < len(to_smem):
            to_smem[k].start()

    forwarded = []

    def forward():
        k = len(forwarded)
        forwarded.append(k)
        to_smem[k].wait()
        to_vmem[k].start()
        fetch(k + 2)

    def act(pos):
        for a in plan.get(pos, ""):
            {"f": forward, "i": issue}[a]()

    def wait(name):
        act(name)
        for cp in waits[name]:
            cp.wait()

    fetch(0)
    fetch(1)
    issue()

    ew = _LANES * H
    for j in range(ew // _CB):
        row = lax.broadcasted_iota(jnp.int32, (_LANES, _CB), 0)
        col = lax.broadcasted_iota(jnp.int32, (_LANES, _CB), 1) + j * _CB
        e_v[:, j * _CB:(j + 1) * _CB] = jnp.where(
            col // H == row, 1.0, 0.0).astype(_BF16)

    def head_mask(rows):
        row = lax.broadcasted_iota(jnp.int32, (rows, _CB), 0)
        col = lax.broadcasted_iota(jnp.int32, (rows, _CB), 1)
        return (col % H) == (row % H)

    def expand(a):
        a4 = jnp.concatenate(
            [jnp.broadcast_to(a[:, u * _LANES:(u + 1) * _LANES], (H, _LANES))
             for u in range(nblk)], axis=0).astype(_BF16)
        mask = head_mask(nblk * H)
        for j in range(ew // _CB):
            xj = jnp.dot(a4, e_v[:, j * _CB:(j + 1) * _CB],
                         preferred_element_type=_F32)
            xj = jnp.where(mask, xj, 0.0).astype(_BF16)
            for u in range(nblk):
                s_v[:, u * ew + j * _CB:u * ew + (j + 1) * _CB] = (
                    xj[u * H:(u + 1) * H, :])

    def rows_of(w_v, r0, n):
        nt = w_v.shape[1]
        g, t = divmod(r0 // 8, nt)
        if t == 0 and n // 8 % nt == 0:
            blk = w_v[g:g + n // 8 // nt]
        else:
            assert t + n // 8 <= nt
            blk = w_v[g, t:t + n // 8]
        return blk.reshape(n, _LANES)

    def per_head_matvec(w_v):
        parts = [
            jnp.dot(s_v[:, u * ew:(u + 1) * ew], rows_of(w_v, u * ew, ew),
                    preferred_element_type=_F32)
            for u in range(nblk)
        ]
        return functools.reduce(lambda a, b: a + b, parts)

    wait("wmod")
    wait("x")
    wait("c")
    cc = c_v[...].astype(_F32)
    silu_c = jnp.broadcast_to(cc * jax.nn.sigmoid(cc), (8, M)).astype(_BF16)
    mod = jnp.dot(silu_c, _untile(wmod_v[...], 6 * M // _LANES),
                  preferred_element_type=_F32)[0:1, :]
    sa, ca, ga, sb, cb, gb = (mod[:, i * M:(i + 1) * M] for i in range(6))
    x0 = x_v[...].astype(_F32)
    h1 = _layernorm(x0) * (1.0 + ca) + sa

    expand(h1)
    wait("wq")
    q = per_head_matvec(wq_v).astype(_BF16)

    wait("wuk")
    scale = float(D) ** -0.5
    mask = head_mask(H)
    for j in range(DC * H // _CB):
        rj = lax.dot_general(q, rows_of(wuk_v, j * _CB, _CB), _NT,
                             preferred_element_type=_F32)
        s_v[:, j * _CB:(j + 1) * _CB] = jnp.where(
            mask, rj * scale, 0.0).astype(_BF16)
    r4 = jnp.concatenate(
        [s_v[:, u * ew:(u + 1) * ew] for u in range(nblk)], axis=0)
    qa4 = lax.dot_general(r4, e_v[...], _NT,
                          preferred_element_type=_F32)
    qa = jnp.concatenate(
        [qa4[u * H:(u + 1) * H, :] for u in range(nblk)], axis=1
    ).astype(_BF16)

    def attend(i, carry):
        m, l, acc = carry
        kv = _untile(ckv_v[:, pl.ds(i * _BT, _BT)], nblk)
        s = lax.dot_general(qa, kv, _NT, preferred_element_type=_F32)
        m_new = jnp.maximum(m, jnp.max(s, axis=1, keepdims=True))
        alpha = jnp.exp(m - m_new)
        p = jnp.exp(s - m_new)
        l = l * alpha + jnp.sum(p, axis=1, keepdims=True)
        acc = acc * alpha + jnp.dot(p.astype(_BF16), kv,
                                    preferred_element_type=_F32)
        return m_new, l, acc

    def attn_step(i, carry):
        for j in range(n_kv - 1):
            if f"kv{j}" in plan:
                pl.when(i == j)(functools.partial(act, f"kv{j}"))
        kv_block(i).wait()
        return attend(i, carry)

    carry = (jnp.full((H, 1), -jnp.inf, _F32), jnp.zeros((H, 1), _F32),
             jnp.zeros((H, DC), _F32))
    wait("kvh")
    carry = lax.fori_loop(0, n_kv - 1, attn_step, carry)
    wait(kv_last)
    _, l, acc = attend(n_kv - 1, carry)

    expand(acc / l)
    wait("wuv")
    ctx = per_head_matvec(wuv_v)

    row = lax.broadcasted_iota(jnp.int32, (H, D), 0)
    lhs = jnp.concatenate(
        [jnp.where(row == h, ctx, 0.0).astype(_BF16) for h in range(H)],
        axis=1)
    wait("wo")
    attn = jnp.sum(jnp.dot(lhs, _untile(wo_v[...], M // _LANES),
                           preferred_element_type=_F32),
                   axis=0, keepdims=True)
    x1 = x0 + ga * attn

    h2 = _layernorm(x1) * (1.0 + cb) + sb
    h2 = jnp.broadcast_to(h2, (8, M)).astype(_BF16)
    wait("wu")
    u = jnp.dot(h2, wu_v[...], preferred_element_type=_F32)
    wait("wg")
    g = jnp.dot(h2, wg_v[...], preferred_element_type=_F32)
    hf = (jax.nn.gelu(g, approximate=True) * u).astype(_BF16)

    n_mxu = wd_parts[0]
    wait("wd0")
    y = jnp.dot(hf[:, :n_mxu], wd_v[:n_mxu, :], preferred_element_type=_F32)
    for j in range(ht_v.shape[0] // _LANES):
        c0 = n_mxu + j * _LANES
        blk = hf[0:1, c0:c0 + _LANES].astype(_F32)
        ht_v[j * _LANES:(j + 1) * _LANES, :] = jnp.broadcast_to(
            blk, (_LANES, _LANES)).T
    sub = lax.broadcasted_iota(jnp.int32, (8, M), 0)
    z = jnp.where(sub == 0, y, 0.0)
    for i in range(1, len(wd_rows)):
        wait(f"wd{i}")
        r0, n = wd_rows[i]
        z_hi = None
        for r in range(r0, r0 + n, 16):
            w = wd_v[r:r + 16, :].astype(_F32)
            hcol = ht_v[r - n_mxu:r - n_mxu + 16, :]
            t = w * jnp.concatenate([hcol] * (M // _LANES), axis=1)
            z = z + t[0:8]
            z_hi = t[8:16] if z_hi is None else z_hi + t[8:16]
        z = z + z_hi
    assert not groups and len(forwarded) == len(to_smem)
    y = jnp.sum(z, axis=0, keepdims=True)
    o_ref[...] = (x1 + gb * y).astype(o_ref.dtype)


@jax.jit
def pallas_adaLN_cond__compressed_kv_cla__glu_gated_geglu__decode_kernel(
    A_x: jax.Array,
    A_c_kv: jax.Array,
    A_w_q: jax.Array,
    A_w_uk: jax.Array,
    A_w_uv: jax.Array,
    A_w_o: jax.Array,
    B_x: jax.Array,
    B_w_gate: jax.Array,
    B_w_up: jax.Array,
    B_w_down: jax.Array,
    c: jax.Array,
    w_mod: jax.Array,
):
    del B_x
    B, SQ, M = A_x.shape
    _, SK, DC = A_c_kv.shape
    _, H, D = A_w_q.shape
    DF = B_w_gate.shape[1]
    assert B == 1 and SQ == 1 and M == DC and D == _LANES

    wd_parts = (1024, 384, 112, 160, 48, 32, 32)
    wd_side = (2, 5)
    wu_side = (64,) * 7 + (16,)
    order = ("kv0 kvh wmod x c wq | kv1 wuk kv2 | kv3 kv4 kv5 kv6 kv7 |"
             "wuv kv8 | kv9 kv10 kv11 kv12 kv13 kv14 kv15 |"
             "wo wu wg wd0 wd1 wd3 wd4 wd6")
    plan = {"wmod": "fi", "wuk": "fi", "kv0": "fi", "kv5": "fi", "kv8": "f",
            "kv10": "fi", "kv14": "f", "wuv": "f", "wo": "ff"}
    first_blk = dict(kv=14, wq=14, wuk=14, wuv=14, wo=14, wmod=16)
    assert sum(wd_parts) == DF and sum(wu_side) < M
    n_sem = len(order.replace("|", " ").split()) + 2 * (
        len(wu_side) + len(wd_side))

    kernel = functools.partial(
        _kernel, n_sem=n_sem, H=H, D=D, M=M, DC=DC, wd_parts=wd_parts,
        wd_side=wd_side, wu_side=wu_side, order=order, plan=plan,
        first_blk=first_blk)

    operands = (
        A_x.reshape(1, M), c, _tiles(w_mod, 6), _tiles(A_w_q, 8),
        _tiles(A_w_uk, 8), _tiles(A_c_kv, 32), _tiles(A_w_uv, 8),
        _tiles(A_w_o, 8), B_w_gate, B_w_up, B_w_down)
    dt = A_x.dtype
    out = pl.pallas_call(
        kernel,
        out_shape=jax.ShapeDtypeStruct((1, M), dt),
        in_specs=[pl.BlockSpec(memory_space=pl.ANY)] * len(operands),
        out_specs=pl.BlockSpec(memory_space=pltpu.VMEM),
        scratch_shapes=[pltpu.VMEM(a.shape, dt) for a in operands] + [
            pltpu.VMEM((_LANES, _LANES * H), _BF16),
            pltpu.VMEM((H, DC * H), _BF16),
            pltpu.VMEM((sum(wd_parts[1:]), _LANES), _F32),
            pltpu.SMEM((3, max(wu_side), DF), dt),
            pltpu.SMEM((sum(wd_parts[i] for i in wd_side), M), dt),
        ],
        compiler_params=pltpu.CompilerParams(
            vmem_limit_bytes=100 * 1024 * 1024),
    )(*operands)
    return out.reshape(B, SQ, M)
```

```python
import functools

import jax
import jax.numpy as jnp
from jax import lax
import jax.experimental.pallas as pl
import jax.experimental.pallas.tpu as pltpu

_F32 = jnp.float32
_BF16 = jnp.bfloat16
_NT = (((1,), (1,)), ((), ()))
_LANES = 128
_CB = 512
_BT = 32


def _layernorm(x, eps=1e-05):
    m = jnp.mean(x, axis=-1, keepdims=True)
    xc = x - m
    v = jnp.mean(xc * xc, axis=-1, keepdims=True)
    return xc / jnp.sqrt(v + eps)


def _row_splits(sizes):
    out, r0 = [], 0
    for n in sizes:
        out.append((r0, n))
        r0 += n
    return out


def _tiles(x, groups):
    x = x.reshape(-1, 8, x.shape[-1] // _LANES, _LANES).transpose(0, 2, 1, 3)
    return x.reshape(groups, -1, 8, _LANES)


def _untile(t, ncol):
    t = t.reshape(-1, ncol, 8, _LANES)
    cols = [t[:, j].reshape(-1, _LANES) for j in range(ncol)]
    return jnp.concatenate(cols, axis=1)


def _kernel(*refs, n_sem, **params):
    pl.run_scoped(
        functools.partial(_body, *refs, **params),
        pltpu.SemaphoreType.DMA((n_sem,)),
    )


def _body(
    x_hbm, c_hbm, wmod_hbm, wq_hbm, wuk_hbm, ckv_hbm, wuv_hbm, wo_hbm,
    wg_hbm, wu_hbm, wd_hbm,
    o_ref,
    x_v, c_v, wmod_v, wq_v, wuk_v, ckv_v, wuv_v, wo_v, wg_v, wu_v, wd_v,
    e_v, s_v, ht_v, wu_s, wd_s, sems,
    *, H, D, M, DC, wd_parts, wd_side, wu_side, order, plan, first_blk,
):
    starts, waits, sem_ids = {}, {}, {}

    def sem(name):
        return sems.at[sem_ids.setdefault(name, len(sem_ids))]

    def add(name, src, dst, rows=None):
        if rows is not None:
            src = src.at[pl.ds(*rows)]
            dst = dst.at[pl.ds(*rows)]
        starts[name] = [pltpu.make_async_copy(src, dst, sem(name))]
        waits[name] = starts[name]

    def add_blocks(name, src, dst):
        nt = src.shape[1]
        cuts = sorted({0, nt, *range(first_blk[name], nt, _BT)})
        starts[name] = [
            pltpu.make_async_copy(src.at[:, pl.ds(a, b - a)],
                                  dst.at[:, pl.ds(a, b - a)], sem(name))
            for a, b in zip(cuts[:-1], cuts[1:])]
        waits[name] = [pltpu.make_async_copy(dst, dst, sem(name))]

    nblk = DC // _LANES
    kv_t = ckv_v.shape[1]
    n_kv = kv_t // _BT
    kv_rot = first_blk["kv"] // nblk * nblk

    def kv_tiles(t0, n, s):
        return pltpu.make_async_copy(
            ckv_hbm.at[:, pl.ds(t0, n)],
            ckv_v.at[:, pl.ds((t0 - kv_rot) % kv_t, n)], s)

    def kv_block(i):
        return pltpu.make_async_copy(
            ckv_hbm.at[:, pl.ds(first_blk["kv"] + _BT * i, _BT)],
            ckv_v.at[:, pl.ds(first_blk["kv"] - kv_rot + _BT * i, _BT)],
            sems.at[i])

    for i in range(n_kv - 1):
        sem(f"kv{i}")
        starts[f"kv{i}"] = [kv_block(i)]
    kv_last = f"kv{n_kv - 1}"
    tail0 = first_blk["kv"] + _BT * (n_kv - 1)
    starts[kv_last] = waits[kv_last] = [
        kv_tiles(tail0, kv_t - tail0, sem(kv_last)),
        kv_tiles(0, kv_rot, sem(kv_last))]
    starts["kvh"] = waits["kvh"] = [
        kv_tiles(kv_rot, first_blk["kv"] - kv_rot, sem("kvh"))]

    wd_rows = _row_splits(wd_parts)
    n_side = sum(wu_side)
    add_blocks("wmod", wmod_hbm, wmod_v)
    add("x", x_hbm, x_v)
    add("c", c_hbm, c_v)
    add_blocks("wq", wq_hbm, wq_v)
    add_blocks("wuk", wuk_hbm, wuk_v)
    add_blocks("wuv", wuv_hbm, wuv_v)
    add_blocks("wo", wo_hbm, wo_v)
    add("wu", wu_hbm, wu_v, (n_side, M - n_side))
    add("wg", wg_hbm, wg_v)
    for i, rows in enumerate(wd_rows):
        if i not in wd_side:
            add(f"wd{i}", wd_hbm, wd_v, rows)

    groups = [g.split() for g in order.split("|")]
    assert sorted(sum(groups, [])) == sorted(starts)

    def issue(g):
        for name in groups[g]:
            for cp in starts[name]:
                cp.start()

    to_smem, to_vmem = [], []

    def add_side(src, stage, dst, rows):
        k = len(to_smem)
        to_smem.append(pltpu.make_async_copy(
            src.at[pl.ds(*rows)], stage, sem(f"to_smem{k}")))
        to_vmem.append(pltpu.make_async_copy(
            stage, dst.at[pl.ds(*rows)], sem(f"to_vmem{k}")))

    n_slot = wu_s.shape[0]
    for k, rows in enumerate(_row_splits(wu_side)):
        add_side(wu_hbm, wu_s.at[k % n_slot, pl.ds(0, rows[1])], wu_v, rows)
    staged = _row_splits([wd_parts[i] for i in wd_side])
    for i, rows in zip(wd_side, staged):
        add_side(wd_hbm, wd_s.at[pl.ds(*rows)], wd_v, wd_rows[i])
        waits[f"wd{i}"] = [to_vmem[-1]]
    waits["wu"] = to_vmem[len(wu_side) - n_slot:len(wu_side)] + waits["wu"]

    def fetch(k):
        if n_slot <= k < len(wu_side):
            to_vmem[k - n_slot].wait()
        if k < len(to_smem):
            to_smem[k].start()

    def forward(k):
        to_smem[k].wait()
        to_vmem[k].start()
        fetch(k + 2)

    count, steps = {"f": 0, "i": 1}, {}
    for pos, actions in plan.items():
        steps[pos] = []
        for a in actions:
            steps[pos].append((forward if a == "f" else issue, count[a]))
            count[a] += 1
    assert count == {"f": len(to_smem), "i": len(groups)}

    def act(pos):
        for action, k in steps.get(pos, ()):
            action(k)

    def wait(name):
        act(name)
        for cp in waits[name]:
            cp.wait()

    fetch(0)
    fetch(1)
    issue(0)

    ew = _LANES * H
    for j in range(ew // _CB):
        row = lax.broadcasted_iota(jnp.int32, (_LANES, _CB), 0)
        col = lax.broadcasted_iota(jnp.int32, (_LANES, _CB), 1) + j * _CB
        e_v[:, j * _CB:(j + 1) * _CB] = jnp.where(
            col // H == row, 1.0, 0.0).astype(_BF16)

    def head_mask(rows):
        row = lax.broadcasted_iota(jnp.int32, (rows, _CB), 0)
        col = lax.broadcasted_iota(jnp.int32, (rows, _CB), 1)
        return (col % H) == (row % H)

    def expand(a):
        a4 = jnp.concatenate(
            [jnp.broadcast_to(a[:, u * _LANES:(u + 1) * _LANES], (H, _LANES))
             for u in range(nblk)], axis=0).astype(_BF16)
        mask = head_mask(nblk * H)
        for j in range(ew // _CB):
            xj = jnp.dot(a4, e_v[:, j * _CB:(j + 1) * _CB],
                         preferred_element_type=_F32)
            xj = jnp.where(mask, xj, 0.0).astype(_BF16)
            for u in range(nblk):
                s_v[:, u * ew + j * _CB:u * ew + (j + 1) * _CB] = (
                    xj[u * H:(u + 1) * H, :])

    def rows_of(w_v, r0, n):
        nt = w_v.shape[1]
        g, t = divmod(r0 // 8, nt)
        if t == 0 and n // 8 % nt == 0:
            blk = w_v[g:g + n // 8 // nt]
        else:
            assert t + n // 8 <= nt
            blk = w_v[g, t:t + n // 8]
        return blk.reshape(n, _LANES)

    def per_head_matvec(w_v):
        parts = [
            jnp.dot(s_v[:, u * ew:(u + 1) * ew], rows_of(w_v, u * ew, ew),
                    preferred_element_type=_F32)
            for u in range(nblk)
        ]
        return functools.reduce(lambda a, b: a + b, parts)

    wait("wmod")
    wait("x")
    wait("c")
    cc = c_v[...].astype(_F32)
    silu_c = jnp.broadcast_to(cc * jax.nn.sigmoid(cc), (8, M)).astype(_BF16)
    mod = jnp.dot(silu_c, _untile(wmod_v[...], 6 * M // _LANES),
                  preferred_element_type=_F32)[0:1, :]
    sa, ca, ga, sb, cb, gb = (mod[:, i * M:(i + 1) * M] for i in range(6))
    x0 = x_v[...].astype(_F32)
    h1 = _layernorm(x0) * (1.0 + ca) + sa

    expand(h1)
    wait("wq")
    q = per_head_matvec(wq_v).astype(_BF16)

    wait("wuk")
    scale = float(D) ** -0.5
    mask = head_mask(H)
    for j in range(DC * H // _CB):
        rj = lax.dot_general(q, rows_of(wuk_v, j * _CB, _CB), _NT,
                             preferred_element_type=_F32)
        s_v[:, j * _CB:(j + 1) * _CB] = jnp.where(
            mask, rj * scale, 0.0).astype(_BF16)
    r4 = jnp.concatenate(
        [s_v[:, u * ew:(u + 1) * ew] for u in range(nblk)], axis=0)
    qa4 = lax.dot_general(r4, e_v[...], _NT,
                          preferred_element_type=_F32)
    qa = jnp.concatenate(
        [qa4[u * H:(u + 1) * H, :] for u in range(nblk)], axis=1
    ).astype(_BF16)

    def attend(i, carry):
        m, l, acc = carry
        kv = _untile(ckv_v[:, pl.ds(i * _BT, _BT)], nblk)
        s = lax.dot_general(qa, kv, _NT, preferred_element_type=_F32)
        m_new = jnp.maximum(m, jnp.max(s, axis=1, keepdims=True))
        alpha = jnp.exp(m - m_new)
        p = jnp.exp(s - m_new)
        l = l * alpha + jnp.sum(p, axis=1, keepdims=True)
        acc = acc * alpha + jnp.dot(p.astype(_BF16), kv,
                                    preferred_element_type=_F32)
        return m_new, l, acc

    def attn_step(i, carry):
        for j in range(n_kv - 1):
            if f"kv{j}" in plan:
                pl.when(i == j)(functools.partial(act, f"kv{j}"))
        kv_block(i).wait()
        return attend(i, carry)

    carry = (jnp.full((H, 1), -jnp.inf, _F32), jnp.zeros((H, 1), _F32),
             jnp.zeros((H, DC), _F32))
    wait("kvh")
    carry = lax.fori_loop(0, n_kv - 1, attn_step, carry)
    wait(kv_last)
    _, l, acc = attend(n_kv - 1, carry)

    expand(acc / l)
    wait("wuv")
    ctx = per_head_matvec(wuv_v)

    row = lax.broadcasted_iota(jnp.int32, (H, D), 0)
    lhs = jnp.concatenate(
        [jnp.where(row == h, ctx, 0.0).astype(_BF16) for h in range(H)],
        axis=1)
    wait("wo")
    attn = jnp.sum(jnp.dot(lhs, _untile(wo_v[...], M // _LANES),
                           preferred_element_type=_F32),
                   axis=0, keepdims=True)
    x1 = x0 + ga * attn

    h2 = _layernorm(x1) * (1.0 + cb) + sb
    h2 = jnp.broadcast_to(h2, (8, M)).astype(_BF16)
    wait("wu")
    u = jnp.dot(h2, wu_v[...], preferred_element_type=_F32)
    wait("wg")
    g = jnp.dot(h2, wg_v[...], preferred_element_type=_F32)
    hf = (jax.nn.gelu(g, approximate=True) * u).astype(_BF16)

    n_mxu = wd_parts[0]
    wait("wd0")
    y = jnp.dot(hf[:, :n_mxu], wd_v[:n_mxu, :], preferred_element_type=_F32)
    for j in range(ht_v.shape[0] // _LANES):
        c0 = n_mxu + j * _LANES
        blk = hf[0:1, c0:c0 + _LANES].astype(_F32)
        ht_v[j * _LANES:(j + 1) * _LANES, :] = jnp.broadcast_to(
            blk, (_LANES, _LANES)).T
    sub = lax.broadcasted_iota(jnp.int32, (8, M), 0)
    z = jnp.where(sub == 0, y, 0.0)
    for i in range(1, len(wd_rows)):
        wait(f"wd{i}")
        r0, n = wd_rows[i]
        z_hi = None
        for r in range(r0, r0 + n, 16):
            w = wd_v[r:r + 16, :].astype(_F32)
            hcol = ht_v[r - n_mxu:r - n_mxu + 16, :]
            t = w * jnp.concatenate([hcol] * (M // _LANES), axis=1)
            z = z + t[0:8]
            z_hi = t[8:16] if z_hi is None else z_hi + t[8:16]
        z = z + z_hi
    y = jnp.sum(z, axis=0, keepdims=True)
    o_ref[...] = (x1 + gb * y).astype(o_ref.dtype)


@jax.jit
def pallas_adaLN_cond__compressed_kv_cla__glu_gated_geglu__decode_kernel(
    A_x: jax.Array,
    A_c_kv: jax.Array,
    A_w_q: jax.Array,
    A_w_uk: jax.Array,
    A_w_uv: jax.Array,
    A_w_o: jax.Array,
    B_x: jax.Array,
    B_w_gate: jax.Array,
    B_w_up: jax.Array,
    B_w_down: jax.Array,
    c: jax.Array,
    w_mod: jax.Array,
):
    del B_x
    B, SQ, M = A_x.shape
    _, SK, DC = A_c_kv.shape
    _, H, D = A_w_q.shape
    DF = B_w_gate.shape[1]
    assert B == 1 and SQ == 1 and M == DC and D == _LANES

    wd_parts = (1024, 384, 112, 160, 48, 32, 32)
    wd_side = (2, 5)
    wu_side = (64,) * 7 + (16,)
    order = ("kv0 kvh wmod x c wq | kv1 wuk kv2 | kv3 kv4 kv5 kv6 kv7 |"
             "wuv kv8 | kv9 kv10 kv11 kv12 kv13 kv14 kv15 |"
             "wo wu wg wd0 wd1 wd3 wd4 wd6")
    plan = {"wmod": "fi", "wuk": "fi", "kv0": "fi", "kv5": "fi", "kv8": "f",
            "kv10": "fi", "kv14": "f", "wuv": "f", "wo": "ff"}
    first_blk = dict(kv=14, wq=14, wuk=14, wuv=14, wo=14, wmod=16)
    assert sum(wd_parts) == DF and sum(wu_side) < M
    n_sem = len(order.replace("|", " ").split()) + 2 * (
        len(wu_side) + len(wd_side))

    kernel = functools.partial(
        _kernel, n_sem=n_sem, H=H, D=D, M=M, DC=DC, wd_parts=wd_parts,
        wd_side=wd_side, wu_side=wu_side, order=order, plan=plan,
        first_blk=first_blk)

    operands = (
        A_x.reshape(1, M), c, _tiles(w_mod, 6), _tiles(A_w_q, 8),
        _tiles(A_w_uk, 8), _tiles(A_c_kv, 32), _tiles(A_w_uv, 8),
        _tiles(A_w_o, 8), B_w_gate, B_w_up, B_w_down)
    dt = A_x.dtype
    out = pl.pallas_call(
        kernel,
        out_shape=jax.ShapeDtypeStruct((1, M), dt),
        in_specs=[pl.BlockSpec(memory_space=pl.ANY)] * len(operands),
        out_specs=pl.BlockSpec(memory_space=pltpu.VMEM),
        scratch_shapes=[pltpu.VMEM(a.shape, dt) for a in operands] + [
            pltpu.VMEM((_LANES, _LANES * H), _BF16),
            pltpu.VMEM((H, DC * H), _BF16),
            pltpu.VMEM((sum(wd_parts[1:]), _LANES), _F32),
            pltpu.SMEM((3, max(wu_side), DF), dt),
            pltpu.SMEM((sum(wd_parts[i] for i in wd_side), M), dt),
        ],
        compiler_params=pltpu.CompilerParams(
            vmem_limit_bytes=100 * 1024 * 1024),
    )(*operands)
    return out.reshape(B, SQ, M)
```
